```python
import jax
import jax.numpy as jnp

def _softmax(x, axis=-1):
    return jax.nn.softmax(x, axis=axis)
def _gelu(x):
    return jax.nn.gelu(x, approximate=True)
def _silu(x):
    return jax.nn.silu(x)
def _sigmoid(x):
    return jax.nn.sigmoid(x)
def _layernorm(x, axis=-1, eps=1e-5):
    m = jnp.mean(x, axis=axis, keepdims=True)
    v = jnp.var(x, axis=axis, keepdims=True)
    return (x - m) / jnp.sqrt(v + eps)
def _scatter_add(tgt, idx, src, axis=0):
    return tgt.at[idx].add(src)
def _segment_sum(src, seg, n):
    return jax.ops.segment_sum(src, seg, n)
class _Rng:
    def __init__(self, key):
        self._k = key
    def _next(self):
        self._k, sub = jax.random.split(self._k)
        return sub
    def normal(self, shape):
        return jax.random.normal(self._next(), shape, dtype=jnp.bfloat16)
    def randint(self, lo, hi, shape):
        return jax.random.randint(self._next(), shape, lo, hi, dtype=jnp.int32)
    def uniform(self, shape, lo=0.0, hi=1.0):
        return jax.random.uniform(self._next(), shape, jnp.bfloat16, lo, hi)
    def permutation(self, n):
        return jax.random.permutation(self._next(), n)


kernel_name = 'concat_heads__sliding_local_dilated__ssm_conv_s5__prompt'

def setup_inputs():
    _rng = _Rng(jax.random.key(int.from_bytes(__import__("os").urandom(4), "little")))
    _w = (lambda a: (lambda t: t.astype(jnp.bfloat16) if jnp.issubdtype(t.dtype, jnp.floating) else t)(jnp.asarray(a)))
    def _A_setup():
        B, S, D = 1, 2048, 448
        return {
            "x": _w((lambda *s: _rng.normal(s) * 0.05)(B, S, D)),
            "wqkv": _w((lambda *s: _rng.normal(s) * 0.05)(D, 3 * D)),
            "wo": _w((lambda *s: _rng.normal(s) * 0.05)(D, D)),
        }
    _A_in = _A_setup()

    def _B_setup():
        B, S, D = 1, 2048, 448
        P = D
        Lambda_re = -0.5 * jnp.exp((lambda *s: _rng.normal(s) * 0.05)(P))
        Lambda_im = (lambda *s: _rng.normal(s) * 0.05)(P) * 1.0
        B_re = (lambda *s: _rng.normal(s) * 0.05)(P, D) * (D ** -0.5)
        B_im = (lambda *s: _rng.normal(s) * 0.05)(P, D) * (D ** -0.5)
        C_re = (lambda *s: _rng.normal(s) * 0.05)(D, P) * (P ** -0.5)
        C_im = (lambda *s: _rng.normal(s) * 0.05)(D, P) * (P ** -0.5)
        log_dt = (lambda *s: _rng.normal(s) * 0.05)(P) * 0.3 - 2.0
        Dskip = (lambda *s: _rng.normal(s) * 0.05)(D)
        return {
            "x": _w((lambda *s: _rng.normal(s) * 0.05)(B, S, D)),
            "Lambda_re": _w(Lambda_re),
            "Lambda_im": _w(Lambda_im),
            "B_re": _w(B_re),
            "B_im": _w(B_im),
            "C_re": _w(C_re),
            "C_im": _w(C_im),
            "log_dt": _w(log_dt),
            "Dskip": _w(Dskip),
        }
    _B_in = _B_setup()

    return {
        "A_x": _A_in["x"],
        "A_wqkv": _A_in["wqkv"],
        "A_wo": _A_in["wo"],
        "B_x": _B_in["x"],
        "B_Lambda_re": _B_in["Lambda_re"],
        "B_Lambda_im": _B_in["Lambda_im"],
        "B_B_re": _B_in["B_re"],
        "B_B_im": _B_in["B_im"],
        "B_C_re": _B_in["C_re"],
        "B_C_im": _B_in["C_im"],
        "B_log_dt": _B_in["log_dt"],
        "B_Dskip": _B_in["Dskip"],
    }

def reference(A_x, A_wqkv, A_wo, B_x, B_Lambda_re, B_Lambda_im, B_B_re, B_B_im, B_C_re, B_C_im, B_log_dt, B_Dskip):
    def _A_ref(x, wqkv, wo):
        B, S, D = x.shape
        H = 16; Dh = D // H
        W, dil = 8, 2
        qkv = (lambda x, *d: x.transpose(*d))((x @ wqkv).reshape(B, S, 3, H, Dh), 2, 0, 3, 1, 4)
        q, k, v = qkv[0], qkv[1], qkv[2]
        scale = Dh ** -0.5
        pos = jnp.arange(S)
        off = jnp.arange(W) * dil
        idx = pos[:, None] - off[None, :]
        mask = idx >= 0
        idx_c = jnp.where(mask, idx, 0).reshape(-1)
        kg = k[:, :, idx_c, :].reshape(B, H, S, W, Dh)
        vg = v[:, :, idx_c, :].reshape(B, H, S, W, Dh)
        logits = jnp.einsum("bhsd,bhswd->bhsw", q, kg) * scale
        logits = jnp.where(mask[None, None, :, :], logits, -1e9)
        attn = _softmax(logits, axis=-1)
        o = jnp.einsum("bhsw,bhswd->bhsd", attn, vg)
        return (lambda x, *d: x.transpose(*d))(o, 0, 2, 1, 3).reshape(B, S, D) @ wo

    def _B_ref(x, Lambda_re, Lambda_im, B_re, B_im, C_re, C_im, log_dt, Dskip):
        Bsz, L, H = x.shape
        Lam = Lambda_re + 1j * Lambda_im
        Bmat = B_re + 1j * B_im
        Cmat = C_re + 1j * C_im
        dt = jnp.exp(log_dt)
        Lam_bar = jnp.exp(dt * Lam)
        B_bar = ((Lam_bar - 1.0) / Lam)[:, None] * Bmat
        Bu = jnp.einsum("bld,pd->blp", x + 0j, B_bar)
        h = jnp.zeros_like(Bu[:, 0, :])
        hs = []
        for t in range(L):
            h = Lam_bar[None, :] * h + Bu[:, t, :]
            hs.append(h)
        hseq = jnp.stack(hs, 1)
        y = 2.0 * jnp.einsum("blp,dp->bld", hseq, Cmat).real + x * Dskip[None, None, :]
        return y

    a = _A_ref(A_x, A_wqkv, A_wo)
    b = _B_ref(B_x, B_Lambda_re, B_Lambda_im, B_B_re, B_B_im, B_C_re, B_C_im, B_log_dt, B_Dskip)
    return jnp.concatenate([a, b], axis=-1)
```

```python
import jax
import jax.numpy as jnp
from jax import lax
import jax.experimental.pallas as pl
import jax.experimental.pallas.tpu as pltpu

S = 2048
D = 448
DP = 512
H = 16
DH = 28
W = 8
DIL = 2
NJ = 16
NL = 128
F32 = jnp.float32
BF16 = jnp.bfloat16


def _cmul(ar, ai, br, bi):
    return ar * br - ai * bi, ar * bi + ai * br


def _col_bcast(row):
    return jnp.broadcast_to(row, (128, DP)).T[:D]


def _re_im_rows(g):
    if g < 6:
        return 64 * g, 384 + 64 * g
    return 768, 832


def _stage_x(raw_ref, xt_ref):
    u = raw_ref.bitcast(jnp.uint32)
    for c in range(S // 128):
        cols = pl.ds(128 * c, 128)
        xt_ref[0, cols, :] = u[0:128, cols].T
        tail = jnp.concatenate(
            [u[128:D // 2, cols], jnp.zeros((256 - D // 2, 128), jnp.uint32)], axis=0)
        xt_ref[1, cols, :] = tail.T


def _x_block(xt_ref, j):
    return jnp.concatenate(
        [pltpu.bitcast(xt_ref[h, pl.ds(j, NL, stride=NJ), :].T, BF16) for h in range(2)], axis=0)


def _kernel(lre_ref, lim_ref, ldt_ref, dsk_ref,
            ax_hbm, wqkv_hbm, wo_hbm, bx_hbm, bre_hbm, bim_hbm, cre_hbm, cim_hbm,
            out_hbm,
            xa_raw, xb_raw, wqkv_raw, wo_raw, bre_raw, bim_raw, cre_raw, cim_raw,
            xa_t, xb_t, xb_p, bbar, cc, wt32, wt, wo32, wot,
            lam_r, lam_i, dsk, bu, st, ht, qt, kk, vv, ot, stage,
            in_sems, out_sems):
    cp_bre = pltpu.make_async_copy(bre_hbm, bre_raw, in_sems.at[0])
    cp_bim = pltpu.make_async_copy(bim_hbm, bim_raw, in_sems.at[1])
    cp_bx = pltpu.make_async_copy(bx_hbm, xb_raw, in_sems.at[2])
    cp_wqkv = pltpu.make_async_copy(wqkv_hbm, wqkv_raw, in_sems.at[3])
    cp_ax = pltpu.make_async_copy(ax_hbm, xa_raw, in_sems.at[4])
    cp_cre = pltpu.make_async_copy(cre_hbm, cre_raw, in_sems.at[5])
    cp_cim = pltpu.make_async_copy(cim_hbm, cim_raw, in_sems.at[6])
    cp_wo = pltpu.make_async_copy(wo_hbm, wo_raw, in_sems.at[7])
    for c in (cp_bre, cp_bim, cp_bx, cp_wqkv, cp_ax, cp_cre, cp_cim, cp_wo):
        c.start()

    def row(ref):
        v = ref[...].astype(F32).reshape(1, D)
        return jnp.concatenate([v, jnp.ones((1, DP - D), F32)], axis=1)

    lr, li = row(lre_ref), row(lim_ref)
    dt = jnp.exp(row(ldt_ref)).astype(BF16).astype(F32)
    mag = jnp.exp(dt * lr)
    ar, ai = mag * jnp.cos(dt * li), mag * jnp.sin(dt * li)
    den = lr * lr + li * li
    cr = ((ar - 1.0) * lr + ai * li) / den
    ci = (ai * lr - (ar - 1.0) * li) / den
    lam_r[...] = _col_bcast(ar)
    lam_i[...] = _col_bcast(-ai)
    cr_b = jnp.tile(_col_bcast(2.0 * cr), (1, 4))[:, :D]
    ci_b = jnp.tile(_col_bcast(2.0 * ci), (1, 4))[:, :D]

    cp_bre.wait()
    cp_bim.wait()
    b_r, b_i = bre_raw[...].astype(F32), bim_raw[...].astype(F32)
    bb_r = (cr_b * b_r - ci_b * b_i).astype(BF16)
    bb_i = (-(cr_b * b_i + ci_b * b_r)).astype(BF16)
    bbar[0:384, 0:D] = bb_r[0:384]
    bbar[384:768, 0:D] = bb_i[0:384]
    bbar[768:832, 0:D] = bb_r[384:D]
    bbar[832:896, 0:D] = bb_i[384:D]
    bbar[:, D:DP] = jnp.zeros((2 * D, DP - D), BF16)

    cp_bx.wait()
    _stage_x(xb_raw, xb_t)

    def scan_step(j, emit):
        for g in range(7):
            ro, io = _re_im_rows(g)
            a_r, a_i = lam_r[64 * g:64 * g + 64], lam_i[64 * g:64 * g + 64]
            p_r, p_i = _cmul(a_r, a_i, st[ro:ro + 64], st[io:io + 64])
            n_r = p_r + bu[j, ro:ro + 64]
            n_i = p_i + bu[j, io:io + 64]
            st[ro:ro + 64] = n_r
            st[io:io + 64] = n_i
            if emit:
                ht[j, ro:ro + 64] = n_r.astype(BF16)
                ht[j, io:io + 64] = n_i.astype(BF16)

    st[...] = jnp.zeros((2 * D, NL), F32)

    @pl.loop(0, NJ)
    def _(j):
        x = _x_block(xb_t, j)
        xb_p[j] = x[0:D]
        bu[j] = jnp.dot(bbar[...], x, preferred_element_type=F32)
        scan_step(j, False)

    lane = lax.broadcasted_iota(jnp.int32, (64, NL), 1)
    for g in range(7):
        ro, io = _re_im_rows(g)
        a_r, a_i = lam_r[64 * g:64 * g + 64], lam_i[64 * g:64 * g + 64]
        for _ in range(4):
            a_r, a_i = _cmul(a_r, a_i, a_r, a_i)
        e_r, e_i = st[ro:ro + 64], st[io:io + 64]
        for k in range(7):
            sh = 1 << k
            s_r = jnp.where(lane >= sh, pltpu.roll(e_r, sh, 1), 0.0)
            s_i = jnp.where(lane >= sh, pltpu.roll(e_i, sh, 1), 0.0)
            p_r, p_i = _cmul(a_r, a_i, s_r, s_i)
            e_r, e_i = e_r + p_r, e_i + p_i
            if k < 6:
                a_r, a_i = _cmul(a_r, a_i, a_r, a_i)
        st[ro:ro + 64] = jnp.where(lane >= 1, pltpu.roll(e_r, 1, 1), 0.0)
        st[io:io + 64] = jnp.where(lane >= 1, pltpu.roll(e_i, 1, 1), 0.0)

    cp_wqkv.wait()
    zpad = jnp.zeros((DP - D, 128), F32)
    for c in range(11):
        lo = min(128 * c, 3 * D - 128)
        blk = jnp.concatenate([wqkv_raw[:, lo:lo + 128].astype(F32), zpad], axis=0)
        for kb in range(4):
            wt32[kb, lo:lo + 128, :] = blk[128 * kb:128 * kb + 128].T
    for t in range(3):
        for d in range(DH):
            for kb in range(4):
                wt[t * D + d * H:t * D + (d + 1) * H, 128 * kb:128 * kb + 128] = (
                    wt32[kb, pl.ds(t * D + d, H, stride=DH), :].astype(BF16))
    cp_ax.wait()
    _stage_x(xa_raw, xa_t)

    lane_d = lax.broadcasted_iota(jnp.int32, (D, NL), 1)

    @pl.loop(0, NJ)
    def _(j):
        x = _x_block(xa_t, j)
        js = (j + 30) % 32
        qt[j] = jnp.dot(wt[0:D], x, preferred_element_type=F32)
        k = jnp.dot(wt[D:2 * D], x, preferred_element_type=F32)
        kk[j + 14] = k
        kk[js] = pltpu.roll(k, 1, 1)
        v = jnp.dot(wt[2 * D:3 * D], x, preferred_element_type=F32)
        vv[j + 14] = v
        vv[js] = jnp.where(lane_d == 0, vv[14], pltpu.roll(v, 1, 1))
        scan_step(j, True)

    cp_cre.wait()
    cp_cim.wait()
    cc[:, 0:384] = cre_raw[:, 0:384]
    cc[:, 384:768] = cim_raw[:, 0:384]
    cc[:, 768:832] = cre_raw[:, 384:D]
    cc[:, 832:896] = cim_raw[:, 384:D]
    cp_wo.wait()
    wo_p = jnp.concatenate([wo_raw[...].astype(F32), jnp.zeros((D, DP - D), F32)], axis=1)
    for kb in range(4):
        wt32[kb, 0:D, :] = wo_p[:, 128 * kb:128 * kb + 128]
        for d in range(DH):
            wo32[d * H:(d + 1) * H, 128 * kb:128 * kb + 128] = wt32[kb, pl.ds(d, H, stride=DH), :]
    wo32[D:DP, :] = jnp.zeros((DP - D, DP), F32)
    wot[...] = wo32[...].T[:D].astype(BF16)

    lane_h = lax.broadcasted_iota(jnp.int32, (H, NL), 1)
    dsk[...] = _col_bcast(row(dsk_ref))
    scale = DH ** -0.5

    def out_copy(j):
        return pltpu.make_async_copy(stage.at[j], out_hbm.at[:, j, :], out_sems.at[j])

    @pl.loop(0, NJ)
    def _(j):
        yt = jnp.dot(cc[...], ht[j], preferred_element_type=F32)
        lg = []
        for w in range(W):
            i = j + 14 - DIL * w
            acc = qt[j, 0:H] * kk[i, 0:H]
            for d in range(1, DH):
                acc = acc + qt[j, d * H:(d + 1) * H] * kk[i, d * H:(d + 1) * H]
            lg.append(jnp.where((lane_h == 0) & (i < 14), -1e9, acc * scale))
        m = lg[0]
        for w in range(1, W):
            m = jnp.maximum(m, lg[w])
        e = [jnp.exp(l - m) for l in lg]
        tot = e[0]
        for w in range(1, W):
            tot = tot + e[w]
        inv = 1.0 / tot
        p = [x * inv for x in e]
        for d in range(DH):
            acc = p[0] * vv[j + 14, d * H:(d + 1) * H]
            for w in range(1, W):
                acc = acc + p[w] * vv[j + 14 - DIL * w, d * H:(d + 1) * H]
            ot[d * H:(d + 1) * H] = acc.astype(BF16)
        at = jnp.dot(wot[:, 0:D], ot[...], preferred_element_type=F32)
        yt = yt + xb_p[j].astype(F32) * dsk[...]
        stage[j] = jnp.concatenate([at, yt], axis=0).T
        out_copy(j).start()

    for j in range(NJ):
        out_copy(j).wait()


@jax.jit
def pallas_concat_heads__sliding_local_dilated__ssm_conv_s5__prompt_kernel(
    A_x, A_wqkv, A_wo, B_x, B_Lambda_re, B_Lambda_im, B_B_re, B_B_im, B_C_re, B_C_im,
    B_log_dt, B_Dskip,
):
    vm = pl.BlockSpec(memory_space=pltpu.VMEM)
    hbm = pl.BlockSpec(memory_space=pltpu.HBM)
    out = pl.pallas_call(
        _kernel,
        in_specs=[vm] * 4 + [hbm] * 8,
        out_specs=hbm,
        out_shape=jax.ShapeDtypeStruct((NL, NJ, 2 * D), F32),
        scratch_shapes=[
            pltpu.VMEM((D, S), BF16), pltpu.VMEM((D, S), BF16),
            pltpu.VMEM((D, 3 * D), BF16), pltpu.VMEM((D, D), BF16),
            pltpu.VMEM((D, D), BF16), pltpu.VMEM((D, D), BF16),
            pltpu.VMEM((D, D), BF16), pltpu.VMEM((D, D), BF16),
            pltpu.VMEM((2, S, 128), jnp.uint32), pltpu.VMEM((2, S, 128), jnp.uint32),
            pltpu.VMEM((NJ, D, NL), BF16),
            pltpu.VMEM((2 * D, DP), BF16), pltpu.VMEM((D, 2 * D), BF16),
            pltpu.VMEM((4, 3 * D, 128), F32), pltpu.VMEM((3 * D, DP), BF16),
            pltpu.VMEM((DP, DP), F32), pltpu.VMEM((D, DP), BF16),
            pltpu.VMEM((D, NL), F32), pltpu.VMEM((D, NL), F32), pltpu.VMEM((D, NL), F32),
            pltpu.VMEM((NJ, 2 * D, NL), F32), pltpu.VMEM((2 * D, NL), F32),
            pltpu.VMEM((NJ, 2 * D, NL), BF16),
            pltpu.VMEM((NJ, D, NL), F32), pltpu.VMEM((32, D, NL), F32),
            pltpu.VMEM((32, D, NL), F32), pltpu.VMEM((D, NL), BF16),
            pltpu.VMEM((NJ, NL, 2 * D), F32),
            pltpu.SemaphoreType.DMA((16,)), pltpu.SemaphoreType.DMA((NJ,)),
        ],
        compiler_params=pltpu.CompilerParams(vmem_limit_bytes=100 * 1024 * 1024),
    )(B_Lambda_re, B_Lambda_im, B_log_dt, B_Dskip,
      A_x[0].T, A_wqkv, A_wo, B_x[0].T, B_B_re, B_B_im, B_C_re, B_C_im)
    return out.reshape(1, S, 2 * D)
```

```python
import jax
import jax.numpy as jnp
from jax import lax
import jax.experimental.pallas as pl
import jax.experimental.pallas.tpu as pltpu

S = 2048
D = 448
DP = 512
HD = D // 2
H = 16
DH = 28
W = 8
DIL = 2
NJ = 16
NL = 128
OG = 2
XS = NJ + 1
OS = 24
F32 = jnp.float32
BF16 = jnp.bfloat16
U32 = jnp.uint32


def _cmul(ar, ai, br, bi):
    return ar * br - ai * bi, ar * bi + ai * br


def _col_bcast(row):
    return jnp.broadcast_to(row, (128, DP)).T[:D]


def _pack(v):
    return pltpu.bitcast(v.astype(BF16), U32)


def _bf(v):
    return pltpu.bitcast(v, BF16)


def _stage_x(raw_ref, xt_ref, c):
    cols = pl.ds(pl.multiple_of(128 * c, 128), 128)
    head = pltpu.bitcast(raw_ref[0:256, cols], U32).T
    tail = jnp.concatenate(
        [pltpu.bitcast(raw_ref[256:D, cols], U32), jnp.zeros(((DP - D) // 2, 128), U32)], axis=0)
    tail = tail.T
    for i in range(128 // NJ):
        dst = pl.ds(c * (128 // NJ * XS) + i * XS, NJ)
        xt_ref[0, dst, :] = head[NJ * i:NJ * i + NJ]
        xt_ref[1, dst, :] = tail[NJ * i:NJ * i + NJ]


def _gather_x(xt_ref, xp_ref, j):
    for h in range(2):
        xp_ref[j, 128 * h:128 * h + 128] = xt_ref[h, pl.ds(j, NL, stride=XS), :].T


def _kernel(lre_ref, lim_ref, ldt_ref, dsk_ref,
            ax_hbm, wqkv_hbm, wo_hbm, bx_hbm, bre_hbm, bim_hbm, cre_hbm, cim_hbm,
            out_hbm,
            xa_raw, xb_raw, wqkv_raw, wo_raw, bre_raw, bim_raw, cre_raw, cim_raw,
            xa_t, xb_t, xa_p, xb_p, bbar, cc, wt32, wt, wo32, wot,
            lam_r, lam_i, dsk, bu, st, et, ct, ht, qt, kk, vv, ot, res, stage,
            in_sems, out_sems):
    cp_bre = pltpu.make_async_copy(bre_hbm, bre_raw, in_sems.at[0])
    cp_bim = pltpu.make_async_copy(bim_hbm, bim_raw, in_sems.at[1])
    cp_bx = [pltpu.make_async_copy(bx_hbm.at[:, pl.ds(512 * i, 512)],
                                   xb_raw.at[:, pl.ds(512 * i, 512)], in_sems.at[8 + i])
             for i in range(4)]
    cp_wqkv = pltpu.make_async_copy(wqkv_hbm, wqkv_raw, in_sems.at[3])
    cp_ax = pltpu.make_async_copy(ax_hbm, xa_raw, in_sems.at[4])
    cp_cre = pltpu.make_async_copy(cre_hbm, cre_raw, in_sems.at[5])
    cp_cim = pltpu.make_async_copy(cim_hbm, cim_raw, in_sems.at[6])
    cp_wo = pltpu.make_async_copy(wo_hbm, wo_raw, in_sems.at[7])
    for c in (*cp_bx, cp_bre, cp_bim, cp_wqkv, cp_ax, cp_cre, cp_cim, cp_wo):
        c.start()

    def row(ref):
        v = ref[...].astype(F32).reshape(1, D)
        return jnp.concatenate([v, jnp.ones((1, DP - D), F32)], axis=1)

    lr, li = row(lre_ref), row(lim_ref)
    dt = jnp.exp(row(ldt_ref)).astype(BF16).astype(F32)
    mag = jnp.exp(dt * lr)
    ar, ai = mag * jnp.cos(dt * li), mag * jnp.sin(dt * li)
    den = lr * lr + li * li
    cr = ((ar - 1.0) * lr + ai * li) / den
    ci = (ai * lr - (ar - 1.0) * li) / den
    lam_r[...] = _col_bcast(ar)
    lam_i[...] = _col_bcast(-ai)
    dsk[...] = _col_bcast(row(dsk_ref))
    cr_b = jnp.tile(_col_bcast(2.0 * cr), (1, 4))
    ci_b = jnp.tile(_col_bcast(2.0 * ci), (1, 4))
    valid = lax.broadcasted_iota(jnp.int32, (1, DP), 1) < D
    pr, pi = jnp.where(valid, ar, 0.0), jnp.where(valid, -ai, 0.0)
    for _ in range(4):
        pr, pi = _cmul(pr, pi, pr, pi)
    blocks = lambda v: [v[:, 128 * i:128 * i + 128] for i in range(4)]
    pw_a = jnp.concatenate(blocks(pr) + blocks(pr), axis=0)
    pw_b = jnp.concatenate(blocks(-pi) + blocks(pi), axis=0)

    for i in range(4):
        cp_bx[i].wait()
        for c in range(4 * i, 4 * i + 4):
            _stage_x(xb_raw, xb_t, c)
    _gather_x(xb_t, xb_p, 0)

    cp_bre.wait()
    cp_bim.wait()
    zcol = jnp.zeros((D, DP - D), F32)
    b_r = jnp.concatenate([bre_raw[...].astype(F32), zcol], axis=1)
    b_i = jnp.concatenate([bim_raw[...].astype(F32), zcol], axis=1)
    bb_r = _pack(cr_b * b_r - ci_b * b_i)
    bb_i = _pack(-(cr_b * b_i + ci_b * b_r))
    for g in range(7):
        bbar[64 * g:64 * g + 32] = bb_r[32 * g:32 * g + 32]
        bbar[64 * g + 32:64 * g + 64] = bb_i[32 * g:32 * g + 32]

    def scan_group(g, src, j_out):
        ro, io = 128 * g, 128 * g + 64
        a_r, a_i = lam_r[64 * g:64 * g + 64], lam_i[64 * g:64 * g + 64]
        p_r, p_i = _cmul(a_r, a_i, st[ro:ro + 64], st[io:io + 64])
        n_r = p_r + src(ro)
        n_i = p_i + src(io)
        st[ro:ro + 64] = n_r
        st[io:io + 64] = n_i
        if j_out is not None:
            ht[j_out, ro // 2:ro // 2 + 32] = _pack(n_r)
            ht[j_out, io // 2:io // 2 + 32] = _pack(n_i)

    st[...] = jnp.zeros((2 * D, NL), F32)

    def p1_base(j):
        x = _bf(xb_p[j])
        _gather_x(xb_t, xb_p, jnp.minimum(j + 1, NJ - 1))
        res = jnp.dot(_bf(bbar[...]), x, preferred_element_type=F32)
        bu[j] = res
        for g in range(7):
            scan_group(g, lambda o: res[o:o + 64], None)

    def wqkv_transpose(lo):
        blk = jnp.concatenate(
            [wqkv_raw[:, pl.ds(lo, 128)].astype(F32), jnp.zeros((DP - D, 128), F32)], axis=0)
        for kb in range(4):
            wt32[kb, pl.ds(lo, 128), :] = blk[128 * kb:128 * kb + 128].T

    def wqkv_gather(idx):
        src = (idx // DH) * D + idx % DH
        dst = pl.ds(pl.multiple_of(idx * (H // 2), H // 2), H // 2)
        for kb in range(4):
            wt[dst, 128 * kb:128 * kb + 128] = _pack(wt32[kb, pl.ds(src, H, stride=DH), :])

    pl.loop(0, 6)(p1_base)
    cp_wqkv.wait()

    @pl.loop(0, 5)
    def _(i):
        p1_base(i + 6)
        for u in range(2):
            wqkv_transpose(pl.multiple_of(256 * i + 128 * u, 128))

    tail = jnp.concatenate(
        [wqkv_raw[:, 1280:3 * D].astype(F32), jnp.zeros((D, 64), F32)], axis=1)
    tail = jnp.concatenate([tail, jnp.zeros((DP - D, 128), F32)], axis=0)
    for kb in range(4):
        wt32[kb, 1280:1408, :] = tail[128 * kb:128 * kb + 128].T
    cp_ax.wait()

    @pl.loop(0, 5)
    def _(i):
        p1_base(i + 11)
        for u in range(17):
            wqkv_gather(jnp.minimum(17 * i + u, 3 * DH - 1))
        for u in range(3):
            _stage_x(xa_raw, xa_t, 3 * i + u)

    _stage_x(xa_raw, xa_t, 15)
    _gather_x(xa_t, xa_p, 0)

    lane_d = lax.broadcasted_iota(jnp.int32, (HD, NL), 1)

    def qkv(j, filler):
        x = _bf(xa_p[j])
        _gather_x(xa_t, xa_p, jnp.minimum(j + 1, NJ - 1))
        js = (j + 30) % 32
        for i, (t, h) in enumerate(((1, 0), (1, 1), (2, 0), (2, 1), (0, 0), (0, 1))):
            r0 = (t * D + h * HD) // 2
            res = jnp.dot(_bf(wt[r0:r0 + HD // 2]), x, preferred_element_type=F32)
            rows = slice(h * HD, (h + 1) * HD)
            if t == 0:
                qt[j, rows] = res
            elif t == 1:
                kk[j + 14, rows] = res
                kk[js, rows] = pltpu.roll(res, 1, 1)
            else:
                vv[j + 14, rows] = res
                vv[js, rows] = jnp.where(lane_d == 0, vv[14, rows], pltpu.roll(res, 1, 1))
            filler(i)

    qkv(0, lambda i: None)
    z64 = jnp.zeros((64, NL), F32)
    for b in range(4):
        for part in range(2):
            lo = st[256 * b + 64 * part:256 * b + 64 * part + 64]
            hi = st[256 * b + 128 + 64 * part:256 * b + 192 + 64 * part] if b < 3 else z64
            et[512 * part + 128 * b:512 * part + 128 * b + 128] = jnp.concatenate([lo, hi], axis=0).T
    c = jnp.zeros((8, 128), F32)
    for l in range(NL):
        ct[pl.ds(l, 8, stride=NL), :] = c
        if l < NL - 1:
            c = (pw_a * c + et[pl.ds(l, 8, stride=NL), :]) + pw_b * pltpu.roll(c, 4, 0)
    for b in range(4):
        for part in range(2):
            t = ct[512 * part + 128 * b:512 * part + 128 * b + 128].T
            st[256 * b + 64 * part:256 * b + 64 * part + 64] = t[0:64]
            if b < 3:
                st[256 * b + 128 + 64 * part:256 * b + 192 + 64 * part] = t[64:128]

    @pl.loop(1, NJ)
    def _(j):
        def filler(i):
            for g in ((0, 1), (2,), (3,), (4,), (5,), (6,))[i]:
                scan_group(g, lambda o: bu[j - 1, o:o + 64], j - 1)
        qkv(j, filler)

    for g in range(7):
        scan_group(g, lambda o: bu[NJ - 1, o:o + 64], NJ - 1)
    cp_cre.wait()
    cp_cim.wait()
    c_r, c_i = pltpu.bitcast(cre_raw[...], U32), pltpu.bitcast(cim_raw[...], U32)
    for g in range(7):
        cc[:, 128 * g:128 * g + 128] = jnp.concatenate(
            [c_r[:, 64 * g:64 * g + 64], c_i[:, 64 * g:64 * g + 64]], axis=1)
    cp_wo.wait()
    wo_p = jnp.concatenate([wo_raw[...].astype(F32), zcol], axis=1)
    for kb in range(4):
        wt32[kb, 0:D, :] = wo_p[:, 128 * kb:128 * kb + 128]
        for d in range(DH):
            wo32[d * H:(d + 1) * H, 128 * kb:128 * kb + 128] = wt32[kb, pl.ds(d, H, stride=DH), :]
    wo32[D:DP, :] = jnp.zeros((DP - D, DP), F32)
    wot[...] = _pack(wo32[...].T[:D])
    ot[D // 2:DP // 2] = jnp.zeros(((DP - D) // 2, NL), U32)

    lane_h = lax.broadcasted_iota(jnp.int32, (H, NL), 1)
    scale = DH ** -0.5

    def out_copies(i):
        rows = pl.ds(i * OG, OG)
        return [pltpu.make_async_copy(stage.at[c, :, rows, :],
                                      out_hbm.at[:, rows, pl.ds(128 * c, 128)],
                                      out_sems.at[i * 7 + c]) for c in range(7)]

    def attend(j, fill_qk, fill_pv):
        acc = [None] * W
        for d in range(DH):
            q = qt[j, d * H:(d + 1) * H]
            for w in range(W):
                t = q * kk[j + 14 - DIL * w, d * H:(d + 1) * H]
                acc[w] = t if d == 0 else acc[w] + t
            fill_qk(d)
        lg = [jnp.where((lane_h == 0) & (j < DIL * w), -1e9, acc[w] * scale) for w in range(W)]
        m = lg[0]
        for w in range(1, W):
            m = jnp.maximum(m, lg[w])
        e = [jnp.exp(l - m) for l in lg]
        tot = e[0]
        for w in range(1, W):
            tot = tot + e[w]
        inv = 1.0 / tot
        p = [x * inv for x in e]
        for d in range(DH):
            fill_pv(d)
            o = p[0] * vv[j + 14, d * H:(d + 1) * H]
            for w in range(1, W):
                o = o + p[w] * vv[j + 14 - DIL * w, d * H:(d + 1) * H]
            ot[d * (H // 2):(d + 1) * (H // 2)] = _pack(o)

    def ssm_out(j, h):
        rows = slice(h * HD, (h + 1) * HD)
        prow = slice(h * HD // 2, (h + 1) * HD // 2)
        y = jnp.dot(_bf(cc[prow]), _bf(ht[j]), preferred_element_type=F32)
        res[j % 2, D + h * HD:D + (h + 1) * HD] = y + _bf(xb_p[j, prow]).astype(F32) * dsk[rows]

    def att_out(j, h):
        prow = slice(h * HD // 2, (h + 1) * HD // 2)
        res[j % 2, h * HD:(h + 1) * HD] = jnp.dot(_bf(wot[prow]), _bf(ot[...]), preferred_element_type=F32)

    def emit(j, c):
        stage.at[c].reshape(NL * OS, 128)[pl.ds(j, NL, stride=OS), :] = res[j % 2, 128 * c:128 * c + 128].T

    def send(j):
        @pl.when((j % OG == OG - 1) & (j >= 0))
        def _():
            for cp in out_copies(j // OG):
                cp.start()

    res[1] = jnp.zeros((2 * D, NL), F32)
    attend(0, lambda d: None, lambda d: ssm_out(0, d // 14) if d % 14 == 0 else None)

    @pl.loop(1, NJ)
    def _(j):
        def fill_qk(d):
            if d in (0, 8):
                att_out(j - 1, d // 8)
            if d % 2 == 0 and d < 14:
                emit((j + NJ - 2) % NJ, (d // 2 + 4) % 7)

        def fill_pv(d):
            if d in (0, 12):
                ssm_out(j, d // 12)

        attend(j, fill_qk, fill_pv)
        send(j - 2)

    att_out(NJ - 1, 0)
    att_out(NJ - 1, 1)
    for c in range(7):
        emit(NJ - 2, c)
    for c in (4, 5, 6, 0, 1, 2, 3):
        emit(NJ - 1, c)
    send(NJ - 1)
    for i in range(NJ // OG):
        for cp in out_copies(i):
            cp.wait()


@jax.jit
def pallas_concat_heads__sliding_local_dilated__ssm_conv_s5__prompt_kernel(
    A_x, A_wqkv, A_wo, B_x, B_Lambda_re, B_Lambda_im, B_B_re, B_B_im, B_C_re, B_C_im,
    B_log_dt, B_Dskip,
):
    vm = pl.BlockSpec(memory_space=pltpu.VMEM)
    hbm = pl.BlockSpec(memory_space=pltpu.HBM)
    out = pl.pallas_call(
        _kernel,
        in_specs=[vm] * 4 + [hbm] * 8,
        out_specs=hbm,
        out_shape=jax.ShapeDtypeStruct((NL, NJ, 2 * D), F32),
        scratch_shapes=[
            pltpu.VMEM((D, S), BF16), pltpu.VMEM((D, S), BF16),
            pltpu.VMEM((D, 3 * D), BF16), pltpu.VMEM((D, D), BF16),
            pltpu.VMEM((D, D), BF16), pltpu.VMEM((D, D), BF16),
            pltpu.VMEM((D, D), BF16), pltpu.VMEM((D, D), BF16),
            pltpu.VMEM((2, NL * XS, 128), U32), pltpu.VMEM((2, NL * XS, 128), U32),
            pltpu.VMEM((NJ, DP // 2, NL), U32), pltpu.VMEM((NJ, DP // 2, NL), U32),
            pltpu.VMEM((D, DP), U32), pltpu.VMEM((D // 2, 2 * D), U32),
            pltpu.VMEM((4, 1408, 128), F32), pltpu.VMEM((3 * D // 2, DP), U32),
            pltpu.VMEM((DP, DP), F32), pltpu.VMEM((D // 2, DP), U32),
            pltpu.VMEM((D, NL), F32), pltpu.VMEM((D, NL), F32), pltpu.VMEM((D, NL), F32),
            pltpu.VMEM((NJ, 2 * D, NL), F32), pltpu.VMEM((2 * D, NL), F32),
            pltpu.VMEM((8 * NL, 128), F32), pltpu.VMEM((8 * NL, 128), F32),
            pltpu.VMEM((NJ, D, NL), U32),
            pltpu.VMEM((NJ, D, NL), F32), pltpu.VMEM((32, D, NL), F32),
            pltpu.VMEM((32, D, NL), F32), pltpu.VMEM((DP // 2, NL), U32),
            pltpu.VMEM((2, 2 * D, NL), F32),
            pltpu.VMEM((7, NL, OS, 128), F32),
            pltpu.SemaphoreType.DMA((16,)), pltpu.SemaphoreType.DMA((7 * NJ // OG,)),
        ],
        compiler_params=pltpu.CompilerParams(vmem_limit_bytes=100 * 1024 * 1024),
    )(B_Lambda_re, B_Lambda_im, B_log_dt, B_Dskip,
      A_x[0].T, A_wqkv, A_wo, B_x[0].T, B_B_re, B_B_im, B_C_re, B_C_im)
    return out.reshape(1, S, 2 * D)
```

```python
import jax
import jax.numpy as jnp
from jax import lax
import jax.experimental.pallas as pl
import jax.experimental.pallas.tpu as pltpu

S = 2048
D = 448
DP = 512
HD = D // 2
H = 16
DH = 28
W = 8
DIL = 2
NJ = 16
NL = 128
OG = 2
XS = NJ + 1
OS = 24
F32 = jnp.float32
BF16 = jnp.bfloat16
U32 = jnp.uint32


def _cmul(ar, ai, br, bi):
    return ar * br - ai * bi, ar * bi + ai * br


def _col_bcast(row):
    return jnp.broadcast_to(row, (128, DP)).T[:D]


def _pack(v):
    return pltpu.bitcast(v.astype(BF16), U32)


def _bf(v):
    return pltpu.bitcast(v, BF16)


def _stage_x(raw_ref, xt_ref, c):
    cols = pl.ds(pl.multiple_of(128 * c, 128), 128)
    head = pltpu.bitcast(raw_ref[0:256, cols], U32).T
    tail = jnp.concatenate(
        [pltpu.bitcast(raw_ref[256:D, cols], U32), jnp.zeros(((DP - D) // 2, 128), U32)], axis=0)
    tail = tail.T
    for i in range(128 // NJ):
        dst = pl.ds(c * (128 // NJ * XS) + i * XS, NJ)
        xt_ref[0, dst, :] = head[NJ * i:NJ * i + NJ]
        xt_ref[1, dst, :] = tail[NJ * i:NJ * i + NJ]


def _gather_x(xt_ref, xp_ref, j):
    for h in range(2):
        xp_ref[j, 128 * h:128 * h + 128] = xt_ref[h, pl.ds(j, NL, stride=XS), :].T


def _kernel(lre_ref, lim_ref, ldt_ref, dsk_ref,
            ax_hbm, wqkv_hbm, wo_hbm, bx_hbm, bre_hbm, bim_hbm, cre_hbm, cim_hbm,
            out_hbm,
            xa_raw, xb_raw, wqkv_raw, wo_raw, bre_raw, bim_raw, cre_raw, cim_raw,
            xa_t, xb_t, xa_p, xb_p, bbar, cc, wt32, wt, wo32, wot,
            lam_r, lam_i, dsk, bu, st, et, ct, ht, qt, kk, vv, ot, res, stage,
            in_sems, out_sems):
    cp_bre = pltpu.make_async_copy(bre_hbm, bre_raw, in_sems.at[0])
    cp_bim = pltpu.make_async_copy(bim_hbm, bim_raw, in_sems.at[1])
    cp_bx = [pltpu.make_async_copy(bx_hbm.at[:, pl.ds(512 * i, 512)],
                                   xb_raw.at[:, pl.ds(512 * i, 512)], in_sems.at[8 + i])
             for i in range(4)]
    cp_wqkv = pltpu.make_async_copy(wqkv_hbm, wqkv_raw, in_sems.at[3])
    cp_ax = pltpu.make_async_copy(ax_hbm, xa_raw, in_sems.at[4])
    cp_cre = pltpu.make_async_copy(cre_hbm, cre_raw, in_sems.at[5])
    cp_cim = pltpu.make_async_copy(cim_hbm, cim_raw, in_sems.at[6])
    cp_wo = pltpu.make_async_copy(wo_hbm, wo_raw, in_sems.at[7])
    for c in (cp_bre, cp_bim, *cp_bx, cp_wqkv, cp_ax, cp_cre, cp_cim, cp_wo):
        c.start()

    def row(ref):
        v = ref[...].astype(F32).reshape(1, D)
        return jnp.concatenate([v, jnp.ones((1, DP - D), F32)], axis=1)

    lr, li = row(lre_ref), row(lim_ref)
    dt = jnp.exp(row(ldt_ref)).astype(BF16).astype(F32)
    mag = jnp.exp(dt * lr)
    ar, ai = mag * jnp.cos(dt * li), mag * jnp.sin(dt * li)
    den = lr * lr + li * li
    cr = ((ar - 1.0) * lr + ai * li) / den
    ci = (ai * lr - (ar - 1.0) * li) / den
    lam_r[...] = _col_bcast(ar)
    lam_i[...] = _col_bcast(-ai)
    dsk[...] = _col_bcast(row(dsk_ref))
    cr_b = jnp.tile(_col_bcast(2.0 * cr), (1, 4))
    ci_b = jnp.tile(_col_bcast(2.0 * ci), (1, 4))
    valid = lax.broadcasted_iota(jnp.int32, (1, DP), 1) < D
    pr, pi = jnp.where(valid, ar, 0.0), jnp.where(valid, -ai, 0.0)
    for _ in range(4):
        pr, pi = _cmul(pr, pi, pr, pi)
    blocks = lambda v: [v[:, 128 * i:128 * i + 128] for i in range(4)]
    pw_a = jnp.concatenate(blocks(pr) + blocks(pr), axis=0)
    pw_b = jnp.concatenate(blocks(-pi) + blocks(pi), axis=0)

    cp_bre.wait()
    cp_bim.wait()
    zcol = jnp.zeros((D, DP - D), F32)

    def make_bbar(g):
        r = slice(64 * g, 64 * g + 64)
        b_r = jnp.concatenate([bre_raw[r].astype(F32), zcol[r]], axis=1)
        b_i = jnp.concatenate([bim_raw[r].astype(F32), zcol[r]], axis=1)
        bbar[64 * g:64 * g + 32] = _pack(cr_b[r] * b_r - ci_b[r] * b_i)
        bbar[64 * g + 32:64 * g + 64] = _pack(-(cr_b[r] * b_i + ci_b[r] * b_r))

    make_bbar(0)
    make_bbar(1)
    for i in range(4):
        cp_bx[i].wait()
        for c in range(4 * i, 4 * i + 4):
            _stage_x(xb_raw, xb_t, c)
        make_bbar(2 + i)
    _gather_x(xb_t, xb_p, 0)
    make_bbar(6)

    def scan_group(g, src, j_out):
        ro, io = 128 * g, 128 * g + 64
        a_r, a_i = lam_r[64 * g:64 * g + 64], lam_i[64 * g:64 * g + 64]
        p_r, p_i = _cmul(a_r, a_i, st[ro:ro + 64], st[io:io + 64])
        n_r = p_r + src(ro)
        n_i = p_i + src(io)
        st[ro:ro + 64] = n_r
        st[io:io + 64] = n_i
        if j_out is not None:
            ht[j_out, ro // 2:ro // 2 + 32] = _pack(n_r)
            ht[j_out, io // 2:io // 2 + 32] = _pack(n_i)

    st[...] = jnp.zeros((2 * D, NL), F32)

    def p1_base(j):
        x = _bf(xb_p[j])
        _gather_x(xb_t, xb_p, jnp.minimum(j + 1, NJ - 1))
        res = jnp.dot(_bf(bbar[...]), x, preferred_element_type=F32)
        bu[j] = res
        for g in range(7):
            scan_group(g, lambda o: res[o:o + 64], None)

    def wqkv_transpose(lo):
        blk = jnp.concatenate(
            [wqkv_raw[:, pl.ds(lo, 128)].astype(F32), jnp.zeros((DP - D, 128), F32)], axis=0)
        for kb in range(4):
            wt32[kb, pl.ds(lo, 128), :] = blk[128 * kb:128 * kb + 128].T

    def wqkv_gather(idx):
        src = (idx // DH) * D + idx % DH
        dst = pl.ds(pl.multiple_of(idx * (H // 2), H // 2), H // 2)
        for kb in range(4):
            wt[dst, 128 * kb:128 * kb + 128] = _pack(wt32[kb, pl.ds(src, H, stride=DH), :])

    pl.loop(0, 6, unroll=3)(p1_base)
    cp_wqkv.wait()

    @pl.loop(0, 5)
    def _(i):
        p1_base(i + 6)
        for u in range(2):
            wqkv_transpose(pl.multiple_of(256 * i + 128 * u, 128))

    tail = jnp.concatenate(
        [wqkv_raw[:, 1280:3 * D].astype(F32), jnp.zeros((D, 64), F32)], axis=1)
    tail = jnp.concatenate([tail, jnp.zeros((DP - D, 128), F32)], axis=0)
    for kb in range(4):
        wt32[kb, 1280:1408, :] = tail[128 * kb:128 * kb + 128].T
    cp_ax.wait()

    @pl.loop(0, 5)
    def _(i):
        p1_base(i + 11)
        for u in range(17):
            wqkv_gather(jnp.minimum(17 * i + u, 3 * DH - 1))
        for u in range(3):
            _stage_x(xa_raw, xa_t, 3 * i + u)

    _stage_x(xa_raw, xa_t, 15)
    _gather_x(xa_t, xa_p, 0)

    lane_d = lax.broadcasted_iota(jnp.int32, (HD, NL), 1)

    def qkv(j, filler):
        x = _bf(xa_p[j])
        _gather_x(xa_t, xa_p, jnp.minimum(j + 1, NJ - 1))
        js = (j + 30) % 32
        for i, (t, h) in enumerate(((1, 0), (1, 1), (2, 0), (2, 1), (0, 0), (0, 1))):
            r0 = (t * D + h * HD) // 2
            res = jnp.dot(_bf(wt[r0:r0 + HD // 2]), x, preferred_element_type=F32)
            rows = slice(h * HD, (h + 1) * HD)
            if t == 0:
                qt[j, rows] = res
            elif t == 1:
                kk[j + 14, rows] = res
                kk[js, rows] = pltpu.roll(res, 1, 1)
            else:
                vv[j + 14, rows] = res
                vv[js, rows] = jnp.where(lane_d == 0, vv[14, rows], pltpu.roll(res, 1, 1))
            filler(i)

    qkv(0, lambda i: None)
    z64 = jnp.zeros((64, NL), F32)
    for b in range(4):
        for part in range(2):
            lo = st[256 * b + 64 * part:256 * b + 64 * part + 64]
            hi = st[256 * b + 128 + 64 * part:256 * b + 192 + 64 * part] if b < 3 else z64
            et[512 * part + 128 * b:512 * part + 128 * b + 128] = jnp.concatenate([lo, hi], axis=0).T
    c = jnp.zeros((8, 128), F32)
    for l in range(NL):
        ct[pl.ds(l, 8, stride=NL), :] = c
        if l < NL - 1:
            c = (pw_a * c + et[pl.ds(l, 8, stride=NL), :]) + pw_b * pltpu.roll(c, 4, 0)
    for b in range(4):
        for part in range(2):
            t = ct[512 * part + 128 * b:512 * part + 128 * b + 128].T
            st[256 * b + 64 * part:256 * b + 64 * part + 64] = t[0:64]
            if b < 3:
                st[256 * b + 128 + 64 * part:256 * b + 192 + 64 * part] = t[64:128]

    @pl.loop(1, NJ, unroll=3)
    def _(j):
        def filler(i):
            for g in ((0, 1), (2,), (3,), (4,), (5,), (6,))[i]:
                scan_group(g, lambda o: bu[j - 1, o:o + 64], j - 1)
        qkv(j, filler)

    for g in range(7):
        scan_group(g, lambda o: bu[NJ - 1, o:o + 64], NJ - 1)
    cp_cre.wait()
    cp_cim.wait()
    c_r, c_i = pltpu.bitcast(cre_raw[...], U32), pltpu.bitcast(cim_raw[...], U32)
    for g in range(7):
        cc[:, 128 * g:128 * g + 128] = jnp.concatenate(
            [c_r[:, 64 * g:64 * g + 64], c_i[:, 64 * g:64 * g + 64]], axis=1)
    cp_wo.wait()
    wo_p = jnp.concatenate([wo_raw[...].astype(F32), zcol], axis=1)
    for kb in range(4):
        wt32[kb, 0:D, :] = wo_p[:, 128 * kb:128 * kb + 128]
        for d in range(DH):
            wo32[d * H:(d + 1) * H, 128 * kb:128 * kb + 128] = wt32[kb, pl.ds(d, H, stride=DH), :]
    wo32[D:DP, :] = jnp.zeros((DP - D, DP), F32)
    wot[...] = _pack(wo32[...].T[:D])
    ot[D // 2:DP // 2] = jnp.zeros(((DP - D) // 2, NL), U32)

    lane_h = lax.broadcasted_iota(jnp.int32, (H, NL), 1)
    scale = DH ** -0.5

    def out_copies(i):
        rows = pl.ds(i * OG, OG)
        return [pltpu.make_async_copy(stage.at[c, :, rows, :],
                                      out_hbm.at[:, rows, pl.ds(128 * c, 128)],
                                      out_sems.at[i * 7 + c]) for c in range(7)]

    def attend(j, fill_qk, fill_pv):
        acc = [None] * W
        for d in range(DH):
            q = qt[j, d * H:(d + 1) * H]
            for w in range(W):
                t = q * kk[j + 14 - DIL * w, d * H:(d + 1) * H]
                acc[w] = t if d == 0 else acc[w] + t
            fill_qk(d)
        lg = [jnp.where((lane_h == 0) & (j < DIL * w), -1e9, acc[w] * scale) for w in range(W)]
        m = lg[0]
        for w in range(1, W):
            m = jnp.maximum(m, lg[w])
        e = [jnp.exp(l - m) for l in lg]
        tot = e[0]
        for w in range(1, W):
            tot = tot + e[w]
        inv = 1.0 / tot
        p = [x * inv for x in e]
        for d in range(DH):
            fill_pv(d)
            o = p[0] * vv[j + 14, d * H:(d + 1) * H]
            for w in range(1, W):
                o = o + p[w] * vv[j + 14 - DIL * w, d * H:(d + 1) * H]
            ot[d * (H // 2):(d + 1) * (H // 2)] = _pack(o)

    def ssm_out(j, h):
        rows = slice(h * HD, (h + 1) * HD)
        prow = slice(h * HD // 2, (h + 1) * HD // 2)
        y = jnp.dot(_bf(cc[prow]), _bf(ht[j]), preferred_element_type=F32)
        res[j % 2, rows] = y + _bf(xb_p[j, prow]).astype(F32) * dsk[rows]

    def att_out(j, h):
        prow = slice(h * HD // 2, (h + 1) * HD // 2)
        qt[NJ + j % 2, h * HD:(h + 1) * HD] = jnp.dot(_bf(wot[prow]), _bf(ot[...]), preferred_element_type=F32)

    def emit(j, c):
        a = j % 2
        if c < 3:
            blk = qt[NJ + a, 128 * c:128 * c + 128]
        elif c == 3:
            blk = jnp.concatenate([qt[NJ + a, 384:D], res[a, 0:64]], axis=0)
        else:
            blk = res[a, 128 * c - D:128 * c + 128 - D]
        stage.at[c].reshape(NL * OS, 128)[pl.ds(j, NL, stride=OS), :] = blk.T

    def send(j):
        @pl.when((j % OG == OG - 1) & (j >= 0))
        def _():
            for cp in out_copies(j // OG):
                cp.start()

    res[1] = jnp.zeros((D, NL), F32)
    qt[NJ + 1] = jnp.zeros((D, NL), F32)
    attend(0, lambda d: None, lambda d: ssm_out(0, d // 14) if d % 14 == 0 else None)

    @pl.loop(1, NJ)
    def _(j):
        def fill_qk(d):
            if d == 0:
                for c in range(7):
                    emit((j + NJ - 2) % NJ, c)
            if d in (13, 27):
                att_out(j - 1, d // 27)

        def fill_pv(d):
            if d in (0, 12):
                ssm_out(j, d // 12)

        attend(j, fill_qk, fill_pv)
        send(j - 2)

    att_out(NJ - 1, 0)
    att_out(NJ - 1, 1)
    for c in range(7):
        emit(NJ - 2, c)
    for c in (4, 5, 6, 0, 1, 2, 3):
        emit(NJ - 1, c)
    send(NJ - 1)
    for i in range(NJ // OG):
        for cp in out_copies(i):
            cp.wait()


@jax.jit
def pallas_concat_heads__sliding_local_dilated__ssm_conv_s5__prompt_kernel(
    A_x, A_wqkv, A_wo, B_x, B_Lambda_re, B_Lambda_im, B_B_re, B_B_im, B_C_re, B_C_im,
    B_log_dt, B_Dskip,
):
    vm = pl.BlockSpec(memory_space=pltpu.VMEM)
    hbm = pl.BlockSpec(memory_space=pltpu.HBM)
    out = pl.pallas_call(
        _kernel,
        in_specs=[vm] * 4 + [hbm] * 8,
        out_specs=hbm,
        out_shape=jax.ShapeDtypeStruct((NL, NJ, 2 * D), F32),
        scratch_shapes=[
            pltpu.VMEM((D, S), BF16), pltpu.VMEM((D, S), BF16),
            pltpu.VMEM((D, 3 * D), BF16), pltpu.VMEM((D, D), BF16),
            pltpu.VMEM((D, D), BF16), pltpu.VMEM((D, D), BF16),
            pltpu.VMEM((D, D), BF16), pltpu.VMEM((D, D), BF16),
            pltpu.VMEM((2, NL * XS, 128), U32), pltpu.VMEM((2, NL * XS, 128), U32),
            pltpu.VMEM((NJ, DP // 2, NL), U32), pltpu.VMEM((NJ, DP // 2, NL), U32),
            pltpu.VMEM((D, DP), U32), pltpu.VMEM((D // 2, 2 * D), U32),
            pltpu.VMEM((4, 1408, 128), F32), pltpu.VMEM((3 * D // 2, DP), U32),
            pltpu.VMEM((DP, DP), F32), pltpu.VMEM((D // 2, DP), U32),
            pltpu.VMEM((D, NL), F32), pltpu.VMEM((D, NL), F32), pltpu.VMEM((D, NL), F32),
            pltpu.VMEM((NJ, 2 * D, NL), F32), pltpu.VMEM((2 * D, NL), F32),
            pltpu.VMEM((8 * NL, 128), F32), pltpu.VMEM((8 * NL, 128), F32),
            pltpu.VMEM((NJ, D, NL), U32),
            pltpu.VMEM((NJ + 2, D, NL), F32), pltpu.VMEM((32, D, NL), F32),
            pltpu.VMEM((32, D, NL), F32), pltpu.VMEM((DP // 2, NL), U32),
            pltpu.VMEM((2, D, NL), F32),
            pltpu.VMEM((7, NL, OS, 128), F32),
            pltpu.SemaphoreType.DMA((16,)), pltpu.SemaphoreType.DMA((7 * NJ // OG,)),
        ],
        compiler_params=pltpu.CompilerParams(vmem_limit_bytes=100 * 1024 * 1024),
    )(B_Lambda_re, B_Lambda_im, B_log_dt, B_Dskip,
      A_x[0].T, A_wqkv, A_wo, B_x[0].T, B_B_re, B_B_im, B_C_re, B_C_im)
    return out.reshape(1, S, 2 * D)
```

```python
import jax
import jax.numpy as jnp
from jax import lax
import jax.experimental.pallas as pl
import jax.experimental.pallas.tpu as pltpu

S = 2048
D = 448
DP = 512
HD = D // 2
H = 16
DH = 28
W = 8
DIL = 2
NJ = 16
NL = 128
OG = 2
XS = NJ + 1
OS = 24
PLAN = ((13, "a", 0, 112), (27, "a", 112, 224), (28, "a", 224, 448), (28, "y", 0, 448))
F32 = jnp.float32
BF16 = jnp.bfloat16
U32 = jnp.uint32


def _cmul(ar, ai, br, bi):
    return ar * br - ai * bi, ar * bi + ai * br


def _col_bcast(row):
    return jnp.broadcast_to(row, (128, DP)).T[:D]


def _pack(v):
    return pltpu.bitcast(v.astype(BF16), U32)


def _bf(v):
    return pltpu.bitcast(v, BF16)


def _stage_x(raw_ref, xt_ref, c):
    cols = pl.ds(pl.multiple_of(128 * c, 128), 128)
    head = pltpu.bitcast(raw_ref[0:256, cols], U32).T
    tail = jnp.concatenate(
        [pltpu.bitcast(raw_ref[256:D, cols], U32), jnp.zeros(((DP - D) // 2, 128), U32)], axis=0)
    tail = tail.T
    for i in range(128 // NJ):
        dst = pl.ds(c * (128 // NJ * XS) + i * XS, NJ)
        xt_ref[0, dst, :] = head[NJ * i:NJ * i + NJ]
        xt_ref[1, dst, :] = tail[NJ * i:NJ * i + NJ]


def _gather_x(xt_ref, xp_ref, j):
    for h in range(2):
        xp_ref[j, 128 * h:128 * h + 128] = xt_ref[h, pl.ds(j, NL, stride=XS), :].T


def _kernel(lre_ref, lim_ref, ldt_ref, dsk_ref,
            ax_hbm, wqkv_hbm, wo_hbm, bx_hbm, bre_hbm, bim_hbm, cre_hbm, cim_hbm,
            out_hbm,
            xa_raw, xb_raw, wqkv_raw, wo_raw, bre_raw, bim_raw, cre_raw, cim_raw,
            xa_t, xb_t, xa_p, xb_p, bbar, cc, wt32, wt, wo32, wot,
            lam_r, lam_i, dsk, bu, st, et, ct, ht, qt, kk, vv, ot, res, stage,
            in_sems, out_sems):
    cp_bre = pltpu.make_async_copy(bre_hbm, bre_raw, in_sems.at[0])
    cp_bim = pltpu.make_async_copy(bim_hbm, bim_raw, in_sems.at[1])
    cp_bx = [pltpu.make_async_copy(bx_hbm.at[:, pl.ds(512 * i, 512)],
                                   xb_raw.at[:, pl.ds(512 * i, 512)], in_sems.at[8 + i])
             for i in range(4)]
    cp_wqkv = pltpu.make_async_copy(wqkv_hbm, wqkv_raw, in_sems.at[3])
    cp_ax = pltpu.make_async_copy(ax_hbm, xa_raw, in_sems.at[4])
    cp_cre = pltpu.make_async_copy(cre_hbm, cre_raw, in_sems.at[5])
    cp_cim = pltpu.make_async_copy(cim_hbm, cim_raw, in_sems.at[6])
    cp_wo = pltpu.make_async_copy(wo_hbm, wo_raw, in_sems.at[7])
    for c in (cp_bre, cp_bim, *cp_bx, cp_wqkv, cp_ax, cp_cre, cp_cim, cp_wo):
        c.start()

    def row(ref):
        v = ref[...].astype(F32).reshape(1, D)
        return jnp.concatenate([v, jnp.ones((1, DP - D), F32)], axis=1)

    lr, li = row(lre_ref), row(lim_ref)
    dt = jnp.exp(row(ldt_ref)).astype(BF16).astype(F32)
    mag = jnp.exp(dt * lr)
    ar, ai = mag * jnp.cos(dt * li), mag * jnp.sin(dt * li)
    den = lr * lr + li * li
    cr = ((ar - 1.0) * lr + ai * li) / den
    ci = (ai * lr - (ar - 1.0) * li) / den
    lam_r[...] = _col_bcast(ar)
    lam_i[...] = _col_bcast(-ai)
    dsk[...] = _col_bcast(row(dsk_ref))
    cr_b = jnp.tile(_col_bcast(2.0 * cr), (1, 4))
    ci_b = jnp.tile(_col_bcast(2.0 * ci), (1, 4))
    valid = lax.broadcasted_iota(jnp.int32, (1, DP), 1) < D
    pr, pi = jnp.where(valid, ar, 0.0), jnp.where(valid, -ai, 0.0)
    for _ in range(4):
        pr, pi = _cmul(pr, pi, pr, pi)
    blocks = lambda v: [v[:, 128 * i:128 * i + 128] for i in range(4)]
    pw_a = jnp.concatenate(blocks(pr) + blocks(pr), axis=0)
    pw_b = jnp.concatenate(blocks(-pi) + blocks(pi), axis=0)

    cp_bre.wait()
    cp_bim.wait()
    zcol = jnp.zeros((D, DP - D), F32)

    def make_bbar(g):
        r = slice(64 * g, 64 * g + 64)
        b_r = jnp.concatenate([bre_raw[r].astype(F32), zcol[r]], axis=1)
        b_i = jnp.concatenate([bim_raw[r].astype(F32), zcol[r]], axis=1)
        bbar[64 * g:64 * g + 32] = _pack(cr_b[r] * b_r - ci_b[r] * b_i)
        bbar[64 * g + 32:64 * g + 64] = _pack(-(cr_b[r] * b_i + ci_b[r] * b_r))

    make_bbar(0)
    make_bbar(1)
    for i in range(4):
        cp_bx[i].wait()
        for c in range(4 * i, 4 * i + 4):
            _stage_x(xb_raw, xb_t, c)
        make_bbar(2 + i)
    _gather_x(xb_t, xb_p, 0)
    make_bbar(6)

    def scan_group(g, src, j_out):
        ro, io = 128 * g, 128 * g + 64
        a_r, a_i = lam_r[64 * g:64 * g + 64], lam_i[64 * g:64 * g + 64]
        p_r, p_i = _cmul(a_r, a_i, st[ro:ro + 64], st[io:io + 64])
        n_r = p_r + src(ro)
        n_i = p_i + src(io)
        st[ro:ro + 64] = n_r
        st[io:io + 64] = n_i
        if j_out is not None:
            ht[j_out, ro // 2:ro // 2 + 32] = _pack(n_r)
            ht[j_out, io // 2:io // 2 + 32] = _pack(n_i)

    st[...] = jnp.zeros((2 * D, NL), F32)

    def p1_base(j):
        x = _bf(xb_p[j])
        _gather_x(xb_t, xb_p, jnp.minimum(j + 1, NJ - 1))
        res = jnp.dot(_bf(bbar[...]), x, preferred_element_type=F32)
        bu[j] = res
        for g in range(7):
            scan_group(g, lambda o: res[o:o + 64], None)

    def wqkv_transpose(lo):
        blk = jnp.concatenate(
            [wqkv_raw[:, pl.ds(lo, 128)].astype(F32), jnp.zeros((DP - D, 128), F32)], axis=0)
        for kb in range(4):
            wt32[kb, pl.ds(lo, 128), :] = blk[128 * kb:128 * kb + 128].T

    def wqkv_gather(idx):
        src = (idx // DH) * D + idx % DH
        dst = pl.ds(pl.multiple_of(idx * (H // 2), H // 2), H // 2)
        for kb in range(4):
            wt[dst, 128 * kb:128 * kb + 128] = _pack(wt32[kb, pl.ds(src, H, stride=DH), :])

    pl.loop(0, 6, unroll=6)(p1_base)
    cp_wqkv.wait()

    @pl.loop(0, 5)
    def _(i):
        p1_base(i + 6)
        for u in range(2):
            wqkv_transpose(pl.multiple_of(256 * i + 128 * u, 128))

    tail = jnp.concatenate(
        [wqkv_raw[:, 1280:3 * D].astype(F32), jnp.zeros((D, 64), F32)], axis=1)
    tail = jnp.concatenate([tail, jnp.zeros((DP - D, 128), F32)], axis=0)
    for kb in range(4):
        wt32[kb, 1280:1408, :] = tail[128 * kb:128 * kb + 128].T
    cp_ax.wait()

    @pl.loop(0, 5)
    def _(i):
        p1_base(i + 11)
        for u in range(17):
            wqkv_gather(jnp.minimum(17 * i + u, 3 * DH - 1))
        for u in range(3):
            _stage_x(xa_raw, xa_t, 3 * i + u)

    _stage_x(xa_raw, xa_t, 15)
    _gather_x(xa_t, xa_p, 0)

    lane_d = lax.broadcasted_iota(jnp.int32, (HD, NL), 1)

    def qkv(j, filler):
        x = _bf(xa_p[j])
        if j + 1 < NJ:
            _gather_x(xa_t, xa_p, j + 1)
        js = (j + 30) % 32
        for i, (t, h) in enumerate(((1, 0), (1, 1), (2, 0), (2, 1), (0, 0), (0, 1))):
            r0 = (t * D + h * HD) // 2
            res = jnp.dot(_bf(wt[r0:r0 + HD // 2]), x, preferred_element_type=F32)
            rows = slice(h * HD, (h + 1) * HD)
            if t == 0:
                qt[j, rows] = res
            elif t == 1:
                kk[j + 14, rows] = res
                kk[js, rows] = pltpu.roll(res, 1, 1)
            else:
                vv[j + 14, rows] = res
                vv[js, rows] = jnp.where(lane_d == 0, vv[14, rows], pltpu.roll(res, 1, 1))
            filler(i)

    qkv(0, lambda i: None)
    z64 = jnp.zeros((64, NL), F32)
    for b in range(4):
        for part in range(2):
            lo = st[256 * b + 64 * part:256 * b + 64 * part + 64]
            hi = st[256 * b + 128 + 64 * part:256 * b + 192 + 64 * part] if b < 3 else z64
            et[512 * part + 128 * b:512 * part + 128 * b + 128] = jnp.concatenate([lo, hi], axis=0).T
    c = jnp.zeros((8, 128), F32)
    for l in range(NL):
        ct[pl.ds(l, 8, stride=NL), :] = c
        if l < NL - 1:
            c = (pw_a * c + et[pl.ds(l, 8, stride=NL), :]) + pw_b * pltpu.roll(c, 4, 0)
    for b in range(4):
        for part in range(2):
            t = ct[512 * part + 128 * b:512 * part + 128 * b + 128].T
            st[256 * b + 64 * part:256 * b + 64 * part + 64] = t[0:64]
            if b < 3:
                st[256 * b + 128 + 64 * part:256 * b + 192 + 64 * part] = t[64:128]

    for j in range(1, NJ):
        def filler(i):
            for g in ((0, 1), (2,), (3,), (4,), (5,), (6,))[i]:
                scan_group(g, lambda o: bu[j - 1, o:o + 64], j - 1)
        qkv(j, filler)

    for g in range(7):
        scan_group(g, lambda o: bu[NJ - 1, o:o + 64], NJ - 1)
    cp_cre.wait()
    cp_cim.wait()
    c_r, c_i = pltpu.bitcast(cre_raw[...], U32), pltpu.bitcast(cim_raw[...], U32)
    for g in range(7):
        cc[:, 128 * g:128 * g + 128] = jnp.concatenate(
            [c_r[:, 64 * g:64 * g + 64], c_i[:, 64 * g:64 * g + 64]], axis=1)
    cp_wo.wait()
    wo_p = jnp.concatenate([wo_raw[...].astype(F32), zcol], axis=1)
    for kb in range(4):
        wt32[kb, 0:D, :] = wo_p[:, 128 * kb:128 * kb + 128]
        for d in range(DH):
            wo32[d * H:(d + 1) * H, 128 * kb:128 * kb + 128] = wt32[kb, pl.ds(d, H, stride=DH), :]
    wo32[D:DP, :] = jnp.zeros((DP - D, DP), F32)
    wot[...] = _pack(wo32[...].T[:D])
    ot[D // 2:DP // 2] = jnp.zeros(((DP - D) // 2, NL), U32)

    lane_h = lax.broadcasted_iota(jnp.int32, (H, NL), 1)
    scale = DH ** -0.5

    def out_copies(i):
        rows = pl.ds(i * OG, OG)
        return [pltpu.make_async_copy(stage.at[c, :, rows, :],
                                      out_hbm.at[:, rows, pl.ds(128 * c, 128)],
                                      out_sems.at[i * 7 + c]) for c in range(7)]

    def attend(j, fill_qk, fill_pv):
        acc = [None] * W
        for d in range(DH):
            q = qt[j, d * H:(d + 1) * H]
            for w in range(W):
                t = q * kk[j + 14 - DIL * w, d * H:(d + 1) * H]
                acc[w] = t if d == 0 else acc[w] + t
            fill_qk(d)
        lg = [jnp.where((lane_h == 0) & (j < DIL * w), -1e9, acc[w] * scale) for w in range(W)]
        m = lg[0]
        for w in range(1, W):
            m = jnp.maximum(m, lg[w])
        e = [jnp.exp(l - m) for l in lg]
        tot = e[0]
        for w in range(1, W):
            tot = tot + e[w]
        inv = 1.0 / tot
        p = [x * inv for x in e]
        for d in range(DH):
            fill_pv(d)
            o = p[0] * vv[j + 14, d * H:(d + 1) * H]
            for w in range(1, W):
                o = o + p[w] * vv[j + 14 - DIL * w, d * H:(d + 1) * H]
            ot[d * (H // 2):(d + 1) * (H // 2)] = _pack(o)

    def ssm_out(j, lo, hi):
        rows = slice(lo, hi)
        prow = slice(lo // 2, hi // 2)
        y = jnp.dot(_bf(cc[prow]), _bf(ht[j]), preferred_element_type=F32)
        res[j % 2, rows] = y + _bf(xb_p[j, prow]).astype(F32) * dsk[rows]

    def att_out(j, lo, hi):
        prow = slice(lo // 2, hi // 2)
        qt[NJ + j % 2, lo:hi] = jnp.dot(_bf(wot[prow]), _bf(ot[...]), preferred_element_type=F32)

    def emit(j, c):
        a = j % 2
        if c < 3:
            blk = qt[NJ + a, 128 * c:128 * c + 128]
        elif c == 3:
            blk = jnp.concatenate([qt[NJ + a, 384:D], res[a, 0:64]], axis=0)
        else:
            blk = res[a, 128 * c - D:128 * c + 128 - D]
        stage.at[c].reshape(NL * OS, 128)[pl.ds(j, NL, stride=OS), :] = blk.T

    def send(j):
        @pl.when((j % OG == OG - 1) & (j >= 0))
        def _():
            for cp in out_copies(j // OG):
                cp.start()

    res[1] = jnp.zeros((D, NL), F32)
    qt[NJ + 1] = jnp.zeros((D, NL), F32)
    attend(0, lambda d: None, lambda d: ssm_out(0, 16 * d, 16 * d + HD) if d % 14 == 0 else None)

    @pl.loop(1, NJ)
    def _(j):
        def fill_qk(d):
            if d == 0:
                for c in range(7):
                    emit((j + NJ - 2) % NJ, c)
            fill_pv(d - DH)

        def fill_pv(d):
            for pos, kind, lo, hi in PLAN:
                if pos == d + DH:
                    if kind == "a":
                        att_out(j - 1, lo, hi)
                    else:
                        ssm_out(j, lo, hi)

        attend(j, fill_qk, fill_pv)
        send(j - 2)

    att_out(NJ - 1, 0, D)
    for c in range(7):
        emit(NJ - 2, c)
    for c in (4, 5, 6, 0, 1, 2, 3):
        emit(NJ - 1, c)
    send(NJ - 1)
    for i in range(NJ // OG):
        for cp in out_copies(i):
            cp.wait()


@jax.jit
def pallas_concat_heads__sliding_local_dilated__ssm_conv_s5__prompt_kernel(
    A_x, A_wqkv, A_wo, B_x, B_Lambda_re, B_Lambda_im, B_B_re, B_B_im, B_C_re, B_C_im,
    B_log_dt, B_Dskip,
):
    vm = pl.BlockSpec(memory_space=pltpu.VMEM)
    hbm = pl.BlockSpec(memory_space=pltpu.HBM)
    out = pl.pallas_call(
        _kernel,
        in_specs=[vm] * 4 + [hbm] * 8,
        out_specs=hbm,
        out_shape=jax.ShapeDtypeStruct((NL, NJ, 2 * D), F32),
        scratch_shapes=[
            pltpu.VMEM((D, S), BF16), pltpu.VMEM((D, S), BF16),
            pltpu.VMEM((D, 3 * D), BF16), pltpu.VMEM((D, D), BF16),
            pltpu.VMEM((D, D), BF16), pltpu.VMEM((D, D), BF16),
            pltpu.VMEM((D, D), BF16), pltpu.VMEM((D, D), BF16),
            pltpu.VMEM((2, NL * XS, 128), U32), pltpu.VMEM((2, NL * XS, 128), U32),
            pltpu.VMEM((NJ, DP // 2, NL), U32), pltpu.VMEM((NJ, DP // 2, NL), U32),
            pltpu.VMEM((D, DP), U32), pltpu.VMEM((D // 2, 2 * D), U32),
            pltpu.VMEM((4, 1408, 128), F32), pltpu.VMEM((3 * D // 2, DP), U32),
            pltpu.VMEM((DP, DP), F32), pltpu.VMEM((D // 2, DP), U32),
            pltpu.VMEM((D, NL), F32), pltpu.VMEM((D, NL), F32), pltpu.VMEM((D, NL), F32),
            pltpu.VMEM((NJ, 2 * D, NL), F32), pltpu.VMEM((2 * D, NL), F32),
            pltpu.VMEM((8 * NL, 128), F32), pltpu.VMEM((8 * NL, 128), F32),
            pltpu.VMEM((NJ, D, NL), U32),
            pltpu.VMEM((NJ + 2, D, NL), F32), pltpu.VMEM((32, D, NL), F32),
            pltpu.VMEM((32, D, NL), F32), pltpu.VMEM((DP // 2, NL), U32),
            pltpu.VMEM((2, D, NL), F32),
            pltpu.VMEM((7, NL, OS, 128), F32),
            pltpu.SemaphoreType.DMA((16,)), pltpu.SemaphoreType.DMA((7 * NJ // OG,)),
        ],
        compiler_params=pltpu.CompilerParams(vmem_limit_bytes=100 * 1024 * 1024),
    )(B_Lambda_re, B_Lambda_im, B_log_dt, B_Dskip,
      A_x[0].T, A_wqkv, A_wo, B_x[0].T, B_B_re, B_B_im, B_C_re, B_C_im)
    return out.reshape(1, S, 2 * D)
```

```python
import jax
import jax.numpy as jnp
from jax import lax
import jax.experimental.pallas as pl
import jax.experimental.pallas.tpu as pltpu

S = 2048
D = 448
DP = 512
HD = D // 2
H = 16
DH = 28
W = 8
DIL = 2
NJ = 16
NL = 128
OG = 2
XS = NJ + 1
OS = 24
PLAN = ((13, "a", 0, 112), (27, "a", 112, 224), (28, "a", 224, 448), (28, "y", 0, 448))
F32 = jnp.float32
BF16 = jnp.bfloat16
U32 = jnp.uint32


def _cmul(ar, ai, br, bi):
    return ar * br - ai * bi, ar * bi + ai * br


def _col_bcast(row):
    return jnp.broadcast_to(row, (128, DP)).T[:D]


def _min(a, b):
    return min(a, b) if isinstance(a, int) else jnp.minimum(a, b)


def _mult(a, n):
    return a if isinstance(a, int) else pl.multiple_of(a, n)


def _pack(v):
    return pltpu.bitcast(v.astype(BF16), U32)


def _bf(v):
    return pltpu.bitcast(v, BF16)


def _stage_x(raw_ref, xt_ref, c):
    cols = pl.ds(_mult(128 * c, 128), 128)
    head = pltpu.bitcast(raw_ref[0:256, cols], U32).T
    tail = jnp.concatenate(
        [pltpu.bitcast(raw_ref[256:D, cols], U32), jnp.zeros(((DP - D) // 2, 128), U32)], axis=0)
    tail = tail.T
    for i in range(128 // NJ):
        dst = pl.ds(c * (128 // NJ * XS) + i * XS, NJ)
        xt_ref[0, dst, :] = head[NJ * i:NJ * i + NJ]
        xt_ref[1, dst, :] = tail[NJ * i:NJ * i + NJ]


def _gather_x(xt_ref, xp_ref, j):
    for h in range(2):
        xp_ref[j, 128 * h:128 * h + 128] = xt_ref[h, pl.ds(j, NL, stride=XS), :].T


def _kernel(lre_ref, lim_ref, ldt_ref, dsk_ref,
            ax_hbm, wqkv_hbm, wo_hbm, bx_hbm, bre_hbm, bim_hbm, cre_hbm, cim_hbm,
            out_hbm,
            xa_raw, xb_raw, wqkv_raw, wo_raw, bre_raw, bim_raw, cre_raw, cim_raw,
            xa_t, xb_t, xa_p, xb_p, bbar, cc, wt32, wt, wo32, wot,
            lam_r, lam_i, dsk, bu, st, et, ct, ht, qt, kk, vv, ot, res, stage,
            in_sems, out_sems):
    cp_bre = pltpu.make_async_copy(bre_hbm, bre_raw, in_sems.at[0])
    cp_bim = pltpu.make_async_copy(bim_hbm, bim_raw, in_sems.at[1])
    cp_bx = [pltpu.make_async_copy(bx_hbm.at[:, pl.ds(512 * i, 512)],
                                   xb_raw.at[:, pl.ds(512 * i, 512)], in_sems.at[8 + i])
             for i in range(4)]
    cp_wqkv = pltpu.make_async_copy(wqkv_hbm, wqkv_raw, in_sems.at[3])
    cp_ax = pltpu.make_async_copy(ax_hbm, xa_raw, in_sems.at[4])
    cp_cre = pltpu.make_async_copy(cre_hbm, cre_raw, in_sems.at[5])
    cp_cim = pltpu.make_async_copy(cim_hbm, cim_raw, in_sems.at[6])
    cp_wo = pltpu.make_async_copy(wo_hbm, wo_raw, in_sems.at[7])
    for c in (cp_bre, cp_bim, *cp_bx, cp_wqkv, cp_ax, cp_cre, cp_cim, cp_wo):
        c.start()

    def row(ref):
        v = ref[...].astype(F32).reshape(1, D)
        return jnp.concatenate([v, jnp.ones((1, DP - D), F32)], axis=1)

    lr, li = row(lre_ref), row(lim_ref)
    dt = jnp.exp(row(ldt_ref)).astype(BF16).astype(F32)
    mag = jnp.exp(dt * lr)
    ar, ai = mag * jnp.cos(dt * li), mag * jnp.sin(dt * li)
    den = lr * lr + li * li
    cr = ((ar - 1.0) * lr + ai * li) / den
    ci = (ai * lr - (ar - 1.0) * li) / den
    lam_r[...] = _col_bcast(ar)
    lam_i[...] = _col_bcast(-ai)
    dsk[...] = _col_bcast(row(dsk_ref))
    cr_b = jnp.tile(_col_bcast(2.0 * cr), (1, 4))
    ci_b = jnp.tile(_col_bcast(2.0 * ci), (1, 4))
    valid = lax.broadcasted_iota(jnp.int32, (1, DP), 1) < D
    pr, pi = jnp.where(valid, ar, 0.0), jnp.where(valid, -ai, 0.0)
    for _ in range(4):
        pr, pi = _cmul(pr, pi, pr, pi)
    blocks = lambda v: [v[:, 128 * i:128 * i + 128] for i in range(4)]
    pw_a = jnp.concatenate(blocks(pr) + blocks(pr), axis=0)
    pw_b = jnp.concatenate(blocks(-pi) + blocks(pi), axis=0)

    cp_bre.wait()
    cp_bim.wait()
    zcol = jnp.zeros((D, DP - D), F32)

    def make_bbar(g):
        r = slice(64 * g, 64 * g + 64)
        b_r = jnp.concatenate([bre_raw[r].astype(F32), zcol[r]], axis=1)
        b_i = jnp.concatenate([bim_raw[r].astype(F32), zcol[r]], axis=1)
        bbar[64 * g:64 * g + 32] = _pack(cr_b[r] * b_r - ci_b[r] * b_i)
        bbar[64 * g + 32:64 * g + 64] = _pack(-(cr_b[r] * b_i + ci_b[r] * b_r))

    make_bbar(0)
    make_bbar(1)
    for i in range(4):
        cp_bx[i].wait()
        for c in range(4 * i, 4 * i + 4):
            _stage_x(xb_raw, xb_t, c)
        make_bbar(2 + i)
    _gather_x(xb_t, xb_p, 0)
    make_bbar(6)

    def scan_group(g, src, j_out):
        ro, io = 128 * g, 128 * g + 64
        a_r, a_i = lam_r[64 * g:64 * g + 64], lam_i[64 * g:64 * g + 64]
        p_r, p_i = _cmul(a_r, a_i, st[ro:ro + 64], st[io:io + 64])
        n_r = p_r + src(ro)
        n_i = p_i + src(io)
        st[ro:ro + 64] = n_r
        st[io:io + 64] = n_i
        if j_out is not None:
            ht[j_out, ro // 2:ro // 2 + 32] = _pack(n_r)
            ht[j_out, io // 2:io // 2 + 32] = _pack(n_i)

    st[...] = jnp.zeros((2 * D, NL), F32)

    def p1_base(j):
        x = _bf(xb_p[j])
        _gather_x(xb_t, xb_p, _min(j + 1, NJ - 1))
        res = jnp.dot(_bf(bbar[...]), x, preferred_element_type=F32)
        bu[j] = res
        for g in range(7):
            scan_group(g, lambda o: res[o:o + 64], None)

    def wqkv_transpose(lo):
        blk = jnp.concatenate(
            [wqkv_raw[:, pl.ds(lo, 128)].astype(F32), jnp.zeros((DP - D, 128), F32)], axis=0)
        for kb in range(4):
            wt32[kb, pl.ds(lo, 128), :] = blk[128 * kb:128 * kb + 128].T

    def wqkv_gather(idx):
        src = (idx // DH) * D + idx % DH
        dst = pl.ds(_mult(idx * (H // 2), H // 2), H // 2)
        for kb in range(4):
            wt[dst, 128 * kb:128 * kb + 128] = _pack(wt32[kb, pl.ds(src, H, stride=DH), :])

    for j in range(6):
        p1_base(j)
    cp_wqkv.wait()

    for i in range(5):
        p1_base(i + 6)
        for u in range(2):
            wqkv_transpose(_mult(256 * i + 128 * u, 128))

    tail = jnp.concatenate(
        [wqkv_raw[:, 1280:3 * D].astype(F32), jnp.zeros((D, 64), F32)], axis=1)
    tail = jnp.concatenate([tail, jnp.zeros((DP - D, 128), F32)], axis=0)
    for kb in range(4):
        wt32[kb, 1280:1408, :] = tail[128 * kb:128 * kb + 128].T
    cp_ax.wait()

    for i in range(5):
        p1_base(i + 11)
        for u in range(17):
            wqkv_gather(_min(17 * i + u, 3 * DH - 1))
        for u in range(3):
            _stage_x(xa_raw, xa_t, 3 * i + u)

    _stage_x(xa_raw, xa_t, 15)
    _gather_x(xa_t, xa_p, 0)

    lane_d = lax.broadcasted_iota(jnp.int32, (HD, NL), 1)

    def qkv(j, filler):
        x = _bf(xa_p[j])
        if j + 1 < NJ:
            _gather_x(xa_t, xa_p, j + 1)
        js = (j + 30) % 32
        for i, (t, h) in enumerate(((1, 0), (1, 1), (2, 0), (2, 1), (0, 0), (0, 1))):
            r0 = (t * D + h * HD) // 2
            res = jnp.dot(_bf(wt[r0:r0 + HD // 2]), x, preferred_element_type=F32)
            rows = slice(h * HD, (h + 1) * HD)
            if t == 0:
                qt[j, rows] = res
            elif t == 1:
                kk[j + 14, rows] = res
                kk[js, rows] = pltpu.roll(res, 1, 1)
            else:
                vv[j + 14, rows] = res
                vv[js, rows] = jnp.where(lane_d == 0, vv[14, rows], pltpu.roll(res, 1, 1))
            filler(i)

    qkv(0, lambda i: None)
    z64 = jnp.zeros((64, NL), F32)
    for b in range(4):
        for part in range(2):
            lo = st[256 * b + 64 * part:256 * b + 64 * part + 64]
            hi = st[256 * b + 128 + 64 * part:256 * b + 192 + 64 * part] if b < 3 else z64
            et[512 * part + 128 * b:512 * part + 128 * b + 128] = jnp.concatenate([lo, hi], axis=0).T
    c = jnp.zeros((8, 128), F32)
    for l in range(NL):
        ct[pl.ds(l, 8, stride=NL), :] = c
        if l < NL - 1:
            c = (pw_a * c + et[pl.ds(l, 8, stride=NL), :]) + pw_b * pltpu.roll(c, 4, 0)
    for b in range(4):
        for part in range(2):
            t = ct[512 * part + 128 * b:512 * part + 128 * b + 128].T
            st[256 * b + 64 * part:256 * b + 64 * part + 64] = t[0:64]
            if b < 3:
                st[256 * b + 128 + 64 * part:256 * b + 192 + 64 * part] = t[64:128]

    for j in range(1, NJ):
        def filler(i):
            for g in ((0, 1), (2,), (3,), (4,), (5,), (6,))[i]:
                scan_group(g, lambda o: bu[j - 1, o:o + 64], j - 1)
        qkv(j, filler)

    for g in range(7):
        scan_group(g, lambda o: bu[NJ - 1, o:o + 64], NJ - 1)
    cp_cre.wait()
    cp_cim.wait()
    c_r, c_i = pltpu.bitcast(cre_raw[...], U32), pltpu.bitcast(cim_raw[...], U32)
    for g in range(7):
        cc[:, 128 * g:128 * g + 128] = jnp.concatenate(
            [c_r[:, 64 * g:64 * g + 64], c_i[:, 64 * g:64 * g + 64]], axis=1)
    cp_wo.wait()
    wo_p = jnp.concatenate([wo_raw[...].astype(F32), zcol], axis=1)
    for kb in range(4):
        wt32[kb, 0:D, :] = wo_p[:, 128 * kb:128 * kb + 128]
        for d in range(DH):
            wo32[d * H:(d + 1) * H, 128 * kb:128 * kb + 128] = wt32[kb, pl.ds(d, H, stride=DH), :]
    wo32[D:DP, :] = jnp.zeros((DP - D, DP), F32)
    wot[...] = _pack(wo32[...].T[:D])
    ot[D // 2:DP // 2] = jnp.zeros(((DP - D) // 2, NL), U32)

    lane_h = lax.broadcasted_iota(jnp.int32, (H, NL), 1)
    scale = DH ** -0.5

    def out_copies(i):
        rows = pl.ds(i * OG, OG)
        return [pltpu.make_async_copy(stage.at[c, :, rows, :],
                                      out_hbm.at[:, rows, pl.ds(128 * c, 128)],
                                      out_sems.at[i * 7 + c]) for c in range(7)]

    def attend(j, fill_qk, fill_pv):
        acc = [None] * W
        for d in range(DH):
            q = qt[j, d * H:(d + 1) * H]
            for w in range(W):
                t = q * kk[j + 14 - DIL * w, d * H:(d + 1) * H]
                acc[w] = t if d == 0 else acc[w] + t
            fill_qk(d)
        lg = [jnp.where((lane_h == 0) & (j < DIL * w), -1e9, acc[w] * scale) for w in range(W)]
        m = lg[0]
        for w in range(1, W):
            m = jnp.maximum(m, lg[w])
        e = [jnp.exp(l - m) for l in lg]
        tot = e[0]
        for w in range(1, W):
            tot = tot + e[w]
        inv = 1.0 / tot
        p = [x * inv for x in e]
        for d in range(DH):
            fill_pv(d)
            o = p[0] * vv[j + 14, d * H:(d + 1) * H]
            for w in range(1, W):
                o = o + p[w] * vv[j + 14 - DIL * w, d * H:(d + 1) * H]
            ot[d * (H // 2):(d + 1) * (H // 2)] = _pack(o)

    def ssm_out(j, lo, hi):
        rows = slice(lo, hi)
        prow = slice(lo // 2, hi // 2)
        y = jnp.dot(_bf(cc[prow]), _bf(ht[j]), preferred_element_type=F32)
        res[j % 2, rows] = y + _bf(xb_p[j, prow]).astype(F32) * dsk[rows]

    def att_out(j, lo, hi):
        prow = slice(lo // 2, hi // 2)
        qt[NJ + j % 2, lo:hi] = jnp.dot(_bf(wot[prow]), _bf(ot[...]), preferred_element_type=F32)

    def emit(j, c):
        a = j % 2
        if c < 3:
            blk = qt[NJ + a, 128 * c:128 * c + 128]
        elif c == 3:
            blk = jnp.concatenate([qt[NJ + a, 384:D], res[a, 0:64]], axis=0)
        else:
            blk = res[a, 128 * c - D:128 * c + 128 - D]
        stage.at[c].reshape(NL * OS, 128)[pl.ds(j, NL, stride=OS), :] = blk.T

    def send(j):
        @pl.when((j % OG == OG - 1) & (j >= 0))
        def _():
            for cp in out_copies(j // OG):
                cp.start()

    res[1] = jnp.zeros((D, NL), F32)
    qt[NJ + 1] = jnp.zeros((D, NL), F32)
    attend(0, lambda d: None, lambda d: ssm_out(0, 16 * d, 16 * d + HD) if d % 14 == 0 else None)

    @pl.loop(1, NJ)
    def _(j):
        def fill_qk(d):
            if d == 0:
                for c in range(7):
                    emit((j + NJ - 2) % NJ, c)
            fill_pv(d - DH)

        def fill_pv(d):
            for pos, kind, lo, hi in PLAN:
                if pos == d + DH:
                    if kind == "a":
                        att_out(j - 1, lo, hi)
                    else:
                        ssm_out(j, lo, hi)

        attend(j, fill_qk, fill_pv)
        send(j - 2)

    att_out(NJ - 1, 0, D)
    for c in range(7):
        emit(NJ - 2, c)
    for c in (4, 5, 6, 0, 1, 2, 3):
        emit(NJ - 1, c)
    send(NJ - 1)
    for i in range(NJ // OG):
        for cp in out_copies(i):
            cp.wait()


@jax.jit
def pallas_concat_heads__sliding_local_dilated__ssm_conv_s5__prompt_kernel(
    A_x, A_wqkv, A_wo, B_x, B_Lambda_re, B_Lambda_im, B_B_re, B_B_im, B_C_re, B_C_im,
    B_log_dt, B_Dskip,
):
    vm = pl.BlockSpec(memory_space=pltpu.VMEM)
    hbm = pl.BlockSpec(memory_space=pltpu.HBM)
    out = pl.pallas_call(
        _kernel,
        in_specs=[vm] * 4 + [hbm] * 8,
        out_specs=hbm,
        out_shape=jax.ShapeDtypeStruct((NL, NJ, 2 * D), F32),
        scratch_shapes=[
            pltpu.VMEM((D, S), BF16), pltpu.VMEM((D, S), BF16),
            pltpu.VMEM((D, 3 * D), BF16), pltpu.VMEM((D, D), BF16),
            pltpu.VMEM((D, D), BF16), pltpu.VMEM((D, D), BF16),
            pltpu.VMEM((D, D), BF16), pltpu.VMEM((D, D), BF16),
            pltpu.VMEM((2, NL * XS, 128), U32), pltpu.VMEM((2, NL * XS, 128), U32),
            pltpu.VMEM((NJ, DP // 2, NL), U32), pltpu.VMEM((NJ, DP // 2, NL), U32),
            pltpu.VMEM((D, DP), U32), pltpu.VMEM((D // 2, 2 * D), U32),
            pltpu.VMEM((4, 1408, 128), F32), pltpu.VMEM((3 * D // 2, DP), U32),
            pltpu.VMEM((DP, DP), F32), pltpu.VMEM((D // 2, DP), U32),
            pltpu.VMEM((D, NL), F32), pltpu.VMEM((D, NL), F32), pltpu.VMEM((D, NL), F32),
            pltpu.VMEM((NJ, 2 * D, NL), F32), pltpu.VMEM((2 * D, NL), F32),
            pltpu.VMEM((8 * NL, 128), F32), pltpu.VMEM((8 * NL, 128), F32),
            pltpu.VMEM((NJ, D, NL), U32),
            pltpu.VMEM((NJ + 2, D, NL), F32), pltpu.VMEM((32, D, NL), F32),
            pltpu.VMEM((32, D, NL), F32), pltpu.VMEM((DP // 2, NL), U32),
            pltpu.VMEM((2, D, NL), F32),
            pltpu.VMEM((7, NL, OS, 128), F32),
            pltpu.SemaphoreType.DMA((16,)), pltpu.SemaphoreType.DMA((7 * NJ // OG,)),
        ],
        compiler_params=pltpu.CompilerParams(vmem_limit_bytes=100 * 1024 * 1024),
    )(B_Lambda_re, B_Lambda_im, B_log_dt, B_Dskip,
      A_x[0].T, A_wqkv, A_wo, B_x[0].T, B_B_re, B_B_im, B_C_re, B_C_im)
    return out.reshape(1, S, 2 * D)
```

```python
import jax
import jax.numpy as jnp
from jax import lax
import jax.experimental.pallas as pl
import jax.experimental.pallas.tpu as pltpu

S = 2048
D = 448
DP = 512
HD = D // 2
H = 16
DH = 28
W = 8
DIL = 2
NJ = 16
NL = 128
OG = 2
XS = NJ + 1
OS = 24
PLAN = ((13, "a", 0, 112), (27, "a", 112, 224), (28, "a", 224, 448), (28, "y", 0, 448))
F32 = jnp.float32
BF16 = jnp.bfloat16
U32 = jnp.uint32


def _cmul(ar, ai, br, bi):
    return ar * br - ai * bi, ar * bi + ai * br


def _col_bcast(row):
    return jnp.broadcast_to(row, (128, DP)).T[:D]


def _min(a, b):
    return min(a, b) if isinstance(a, int) else jnp.minimum(a, b)


def _mult(a, n):
    return a if isinstance(a, int) else pl.multiple_of(a, n)


def _pack(v):
    return pltpu.bitcast(v.astype(BF16), U32)


def _bf(v):
    return pltpu.bitcast(v, BF16)


def _stage_x(raw_ref, xt_ref, c):
    cols = pl.ds(_mult(128 * c, 128), 128)
    head = pltpu.bitcast(raw_ref[0:256, cols], U32).T
    tail = jnp.concatenate(
        [pltpu.bitcast(raw_ref[256:D, cols], U32), jnp.zeros(((DP - D) // 2, 128), U32)], axis=0)
    tail = tail.T
    for i in range(128 // NJ):
        dst = pl.ds(c * (128 // NJ * XS) + i * XS, NJ)
        xt_ref[0, dst, :] = head[NJ * i:NJ * i + NJ]
        xt_ref[1, dst, :] = tail[NJ * i:NJ * i + NJ]


def _gather_x(xt_ref, xp_ref, j):
    for h in range(2):
        xp_ref[j, 128 * h:128 * h + 128] = xt_ref[h, pl.ds(j, NL, stride=XS), :].T


def _kernel(lre_ref, lim_ref, ldt_ref, dsk_ref,
            ax_hbm, wqkv_hbm, wo_hbm, bx_hbm, bre_hbm, bim_hbm, cre_hbm, cim_hbm,
            out_hbm,
            xa_raw, xb_raw, wqkv_raw, wo_raw, bre_raw, bim_raw, cre_raw, cim_raw,
            xa_t, xb_t, xa_p, xb_p, bbar, cc, wt32, wt, wo32, wot,
            lam_r, lam_i, dsk, bu, st, et, ct, ht, qt, kk, vv, ot, res, stage,
            in_sems, out_sems):
    cp_bre = pltpu.make_async_copy(bre_hbm, bre_raw, in_sems.at[0])
    cp_bim = pltpu.make_async_copy(bim_hbm, bim_raw, in_sems.at[1])
    cp_bx = [pltpu.make_async_copy(bx_hbm.at[:, pl.ds(512 * i, 512)],
                                   xb_raw.at[:, pl.ds(512 * i, 512)], in_sems.at[8 + i])
             for i in range(4)]
    cp_wqkv = pltpu.make_async_copy(wqkv_hbm, wqkv_raw, in_sems.at[3])
    cp_ax = pltpu.make_async_copy(ax_hbm, xa_raw, in_sems.at[4])
    cp_cre = pltpu.make_async_copy(cre_hbm, cre_raw, in_sems.at[5])
    cp_cim = pltpu.make_async_copy(cim_hbm, cim_raw, in_sems.at[6])
    cp_wo = pltpu.make_async_copy(wo_hbm, wo_raw, in_sems.at[7])
    for c in (*cp_bx[:2], cp_bre, cp_bim, *cp_bx[2:], cp_wqkv, cp_ax, cp_cre, cp_cim, cp_wo):
        c.start()

    def row(ref):
        v = ref[...].astype(F32).reshape(1, D)
        return jnp.concatenate([v, jnp.ones((1, DP - D), F32)], axis=1)

    lr, li = row(lre_ref), row(lim_ref)
    dt = jnp.exp(row(ldt_ref)).astype(BF16).astype(F32)
    mag = jnp.exp(dt * lr)
    ar, ai = mag * jnp.cos(dt * li), mag * jnp.sin(dt * li)
    den = lr * lr + li * li
    cr = ((ar - 1.0) * lr + ai * li) / den
    ci = (ai * lr - (ar - 1.0) * li) / den
    lam_r[...] = _col_bcast(ar)
    lam_i[...] = _col_bcast(ai)
    valid = lax.broadcasted_iota(jnp.int32, (1, DP), 1) < D
    pr, pi = jnp.where(valid, ar, 0.0), jnp.where(valid, ai, 0.0)
    for _ in range(4):
        pr, pi = _cmul(pr, pi, pr, pi)
    blocks = lambda v: [v[:, 128 * i:128 * i + 128] for i in range(4)]
    pw_a = jnp.concatenate(blocks(pr) + blocks(pr), axis=0)
    pw_b = jnp.concatenate(blocks(-pi) + blocks(pi), axis=0)

    zcol = jnp.zeros((D, DP - D), F32)

    def make_bbar(g):
        for part, raw in enumerate((bre_raw, bim_raw)):
            u = pltpu.bitcast(raw[64 * g:64 * g + 64], U32)
            bbar[64 * g + 32 * part:64 * g + 32 * part + 32] = jnp.concatenate(
                [u, jnp.zeros((32, DP - D), U32)], axis=1)

    for i in range(4):
        cp_bx[i].wait()
        if i == 2:
            cp_bre.wait()
            cp_bim.wait()
        for c in range(4 * i, 4 * i + 4):
            _stage_x(xb_raw, xb_t, c)
        if i == 2:
            for g in range(7):
                make_bbar(g)
    _gather_x(xb_t, xb_p, 0)

    def scan_group(g, src, j_out):
        ro, io = 128 * g, 128 * g + 64
        a_r, a_i = lam_r[64 * g:64 * g + 64], lam_i[64 * g:64 * g + 64]
        p_r, p_i = _cmul(a_r, a_i, st[ro:ro + 64], st[io:io + 64])
        n_r = p_r + src(ro)
        n_i = p_i + src(io)
        st[ro:ro + 64] = n_r
        st[io:io + 64] = n_i
        if j_out is not None:
            ht[j_out, ro // 2:ro // 2 + 32] = _pack(n_r)
            ht[j_out, io // 2:io // 2 + 32] = _pack(n_i)

    st[...] = jnp.zeros((2 * D, NL), F32)

    def p1_base(j):
        x = _bf(xb_p[j])
        _gather_x(xb_t, xb_p, _min(j + 1, NJ - 1))
        res = jnp.dot(_bf(bbar[...]), x, preferred_element_type=F32)
        bu[j] = res
        for g in range(7):
            scan_group(g, lambda o: res[o:o + 64], None)

    def wqkv_transpose(lo):
        blk = jnp.concatenate(
            [wqkv_raw[:, pl.ds(lo, 128)].astype(F32), jnp.zeros((DP - D, 128), F32)], axis=0)
        for kb in range(4):
            wt32[kb, pl.ds(lo, 128), :] = blk[128 * kb:128 * kb + 128].T

    def wqkv_gather(idx):
        src = (idx // DH) * D + idx % DH
        dst = pl.ds(_mult(idx * (H // 2), H // 2), H // 2)
        for kb in range(4):
            wt[dst, 128 * kb:128 * kb + 128] = _pack(wt32[kb, pl.ds(src, H, stride=DH), :])

    for j in range(6):
        p1_base(j)
    cp_wqkv.wait()

    for i in range(5):
        p1_base(i + 6)
        for u in range(2):
            wqkv_transpose(_mult(256 * i + 128 * u, 128))

    tail = jnp.concatenate(
        [wqkv_raw[:, 1280:3 * D].astype(F32), jnp.zeros((D, 64), F32)], axis=1)
    tail = jnp.concatenate([tail, jnp.zeros((DP - D, 128), F32)], axis=0)
    for kb in range(4):
        wt32[kb, 1280:1408, :] = tail[128 * kb:128 * kb + 128].T
    cp_ax.wait()

    for i in range(5):
        p1_base(i + 11)
        for u in range(17):
            wqkv_gather(_min(17 * i + u, 3 * DH - 1))
        for u in range(3):
            _stage_x(xa_raw, xa_t, 3 * i + u)

    cp_cre.wait()
    cp_cim.wait()
    _stage_x(xa_raw, xa_t, 15)
    _gather_x(xa_t, xa_p, 0)

    lane_d = lax.broadcasted_iota(jnp.int32, (HD, NL), 1)

    def qkv(j, filler):
        x = _bf(xa_p[j])
        if j + 1 < NJ:
            _gather_x(xa_t, xa_p, j + 1)
        js = (j + 30) % 32
        for i, (t, h) in enumerate(((1, 0), (1, 1), (2, 0), (2, 1), (0, 0), (0, 1))):
            r0 = (t * D + h * HD) // 2
            res = jnp.dot(_bf(wt[r0:r0 + HD // 2]), x, preferred_element_type=F32)
            rows = slice(h * HD, (h + 1) * HD)
            if t == 0:
                qt[j, rows] = res
            elif t == 1:
                kk[j + 14, rows] = res
                kk[js, rows] = pltpu.roll(res, 1, 1)
            else:
                vv[j + 14, rows] = res
                vv[js, rows] = jnp.where(lane_d == 0, vv[14, rows], pltpu.roll(res, 1, 1))
            filler(i)

    qkv(0, lambda i: None)
    z64 = jnp.zeros((64, NL), F32)
    for b in range(4):
        for part in range(2):
            lo = st[256 * b + 64 * part:256 * b + 64 * part + 64]
            hi = st[256 * b + 128 + 64 * part:256 * b + 192 + 64 * part] if b < 3 else z64
            et[512 * part + 128 * b:512 * part + 128 * b + 128] = jnp.concatenate([lo, hi], axis=0).T
    c = jnp.zeros((8, 128), F32)
    for l in range(NL):
        ct[pl.ds(l, 8, stride=NL), :] = c
        if l < NL - 1:
            c = (pw_a * c + et[pl.ds(l, 8, stride=NL), :]) + pw_b * pltpu.roll(c, 4, 0)
    for b in range(4):
        for part in range(2):
            t = ct[512 * part + 128 * b:512 * part + 128 * b + 128].T
            st[256 * b + 64 * part:256 * b + 64 * part + 64] = t[0:64]
            if b < 3:
                st[256 * b + 128 + 64 * part:256 * b + 192 + 64 * part] = t[64:128]

    dsk[...] = _col_bcast(row(dsk_ref))

    def make_cc(r):
        x_r, x_i = cre_raw[r:r + 64].astype(F32), cim_raw[r:r + 64].astype(F32)
        g_r, g_i = 2.0 * cr[:, :D], 2.0 * ci[:, :D]
        c_r = _pack(g_r * x_r - g_i * x_i)
        c_i = _pack(-(g_r * x_i + g_i * x_r))
        for g in range(7):
            cc[r // 2:r // 2 + 32, 128 * g:128 * g + 128] = jnp.concatenate(
                [c_r[:, 64 * g:64 * g + 64], c_i[:, 64 * g:64 * g + 64]], axis=1)

    for j in range(1, NJ):
        def filler(i):
            for g in ((0, 1), (2,), (3,), (4,), (5,), (6,))[i]:
                scan_group(g, lambda o: bu[j - 1, o:o + 64], j - 1)
        qkv(j, filler)
        if j % 2 == 0:
            make_cc(32 * (j - 2))

    for g in range(7):
        scan_group(g, lambda o: bu[NJ - 1, o:o + 64], NJ - 1)
    cp_wo.wait()
    wo_p = jnp.concatenate([wo_raw[...].astype(F32), zcol], axis=1)
    for kb in range(4):
        wt32[kb, 0:D, :] = wo_p[:, 128 * kb:128 * kb + 128]
        for d in range(DH):
            wo32[d * H:(d + 1) * H, 128 * kb:128 * kb + 128] = wt32[kb, pl.ds(d, H, stride=DH), :]
    wo32[D:DP, :] = jnp.zeros((DP - D, DP), F32)
    wot[...] = _pack(wo32[...].T[:D])
    ot[D // 2:DP // 2] = jnp.zeros(((DP - D) // 2, NL), U32)

    lane_h = lax.broadcasted_iota(jnp.int32, (H, NL), 1)
    scale = DH ** -0.5

    def out_copies(i):
        rows = pl.ds(i * OG, OG)
        return [pltpu.make_async_copy(stage.at[c, :, rows, :],
                                      out_hbm.at[:, rows, pl.ds(128 * c, 128)],
                                      out_sems.at[i * 7 + c]) for c in range(7)]

    def attend(j, fill_qk, fill_pv):
        acc = [None] * W
        for d in range(DH):
            q = qt[j, d * H:(d + 1) * H]
            for w in range(W):
                t = q * kk[j + 14 - DIL * w, d * H:(d + 1) * H]
                acc[w] = t if d == 0 else acc[w] + t
            fill_qk(d)
        lg = [jnp.where((lane_h == 0) & (j < DIL * w), -1e9, acc[w] * scale) for w in range(W)]
        m = lg[0]
        for w in range(1, W):
            m = jnp.maximum(m, lg[w])
        e = [jnp.exp(l - m) for l in lg]
        tot = e[0]
        for w in range(1, W):
            tot = tot + e[w]
        inv = 1.0 / tot
        p = [x * inv for x in e]
        for d in range(DH):
            fill_pv(d)
            o = p[0] * vv[j + 14, d * H:(d + 1) * H]
            for w in range(1, W):
                o = o + p[w] * vv[j + 14 - DIL * w, d * H:(d + 1) * H]
            ot[d * (H // 2):(d + 1) * (H // 2)] = _pack(o)

    def ssm_out(j, lo, hi):
        rows = slice(lo, hi)
        prow = slice(lo // 2, hi // 2)
        y = jnp.dot(_bf(cc[prow]), _bf(ht[j]), preferred_element_type=F32)
        res[j % 2, rows] = y + _bf(xb_p[j, prow]).astype(F32) * dsk[rows]

    def att_out(j, lo, hi):
        prow = slice(lo // 2, hi // 2)
        qt[NJ + j % 2, lo:hi] = jnp.dot(_bf(wot[prow]), _bf(ot[...]), preferred_element_type=F32)

    def emit(j, c):
        a = j % 2
        if c < 3:
            blk = qt[NJ + a, 128 * c:128 * c + 128]
        elif c == 3:
            blk = jnp.concatenate([qt[NJ + a, 384:D], res[a, 0:64]], axis=0)
        else:
            blk = res[a, 128 * c - D:128 * c + 128 - D]
        stage.at[c].reshape(NL * OS, 128)[pl.ds(j, NL, stride=OS), :] = blk.T

    def send(j):
        @pl.when((j % OG == OG - 1) & (j >= 0))
        def _():
            for cp in out_copies(j // OG):
                cp.start()

    res[1] = jnp.zeros((D, NL), F32)
    qt[NJ + 1] = jnp.zeros((D, NL), F32)
    attend(0, lambda d: None, lambda d: ssm_out(0, 16 * d, 16 * d + HD) if d % 14 == 0 else None)

    @pl.loop(1, NJ)
    def _(j):
        def fill_qk(d):
            if d == 0:
                for c in range(7):
                    emit((j + NJ - 2) % NJ, c)
            fill_pv(d - DH)

        def fill_pv(d):
            for pos, kind, lo, hi in PLAN:
                if pos == d + DH:
                    if kind == "a":
                        att_out(j - 1, lo, hi)
                    else:
                        ssm_out(j, lo, hi)

        attend(j, fill_qk, fill_pv)
        send(j - 2)

    att_out(NJ - 1, 0, D)
    for c in range(7):
        emit(NJ - 2, c)
    for c in (4, 5, 6, 0, 1, 2, 3):
        emit(NJ - 1, c)
    send(NJ - 1)
    for i in range(NJ // OG):
        for cp in out_copies(i):
            cp.wait()


@jax.jit
def pallas_concat_heads__sliding_local_dilated__ssm_conv_s5__prompt_kernel(
    A_x, A_wqkv, A_wo, B_x, B_Lambda_re, B_Lambda_im, B_B_re, B_B_im, B_C_re, B_C_im,
    B_log_dt, B_Dskip,
):
    vm = pl.BlockSpec(memory_space=pltpu.VMEM)
    hbm = pl.BlockSpec(memory_space=pltpu.HBM)
    out = pl.pallas_call(
        _kernel,
        in_specs=[vm] * 4 + [hbm] * 8,
        out_specs=hbm,
        out_shape=jax.ShapeDtypeStruct((NL, NJ, 2 * D), F32),
        scratch_shapes=[
            pltpu.VMEM((D, S), BF16), pltpu.VMEM((D, S), BF16),
            pltpu.VMEM((D, 3 * D), BF16), pltpu.VMEM((D, D), BF16),
            pltpu.VMEM((D, D), BF16), pltpu.VMEM((D, D), BF16),
            pltpu.VMEM((D, D), BF16), pltpu.VMEM((D, D), BF16),
            pltpu.VMEM((2, NL * XS, 128), U32), pltpu.VMEM((2, NL * XS, 128), U32),
            pltpu.VMEM((NJ, DP // 2, NL), U32), pltpu.VMEM((NJ, DP // 2, NL), U32),
            pltpu.VMEM((D, DP), U32), pltpu.VMEM((D // 2, 2 * D), U32),
            pltpu.VMEM((4, 1408, 128), F32), pltpu.VMEM((3 * D // 2, DP), U32),
            pltpu.VMEM((DP, DP), F32), pltpu.VMEM((D // 2, DP), U32),
            pltpu.VMEM((D, NL), F32), pltpu.VMEM((D, NL), F32), pltpu.VMEM((D, NL), F32),
            pltpu.VMEM((NJ, 2 * D, NL), F32), pltpu.VMEM((2 * D, NL), F32),
            pltpu.VMEM((8 * NL, 128), F32), pltpu.VMEM((8 * NL, 128), F32),
            pltpu.VMEM((NJ, D, NL), U32),
            pltpu.VMEM((NJ + 2, D, NL), F32), pltpu.VMEM((32, D, NL), F32),
            pltpu.VMEM((32, D, NL), F32), pltpu.VMEM((DP // 2, NL), U32),
            pltpu.VMEM((2, D, NL), F32),
            pltpu.VMEM((7, NL, OS, 128), F32),
            pltpu.SemaphoreType.DMA((16,)), pltpu.SemaphoreType.DMA((7 * NJ // OG,)),
        ],
        compiler_params=pltpu.CompilerParams(vmem_limit_bytes=100 * 1024 * 1024),
    )(B_Lambda_re, B_Lambda_im, B_log_dt, B_Dskip,
      A_x[0].T, A_wqkv, A_wo, B_x[0].T, B_B_re, B_B_im, B_C_re, B_C_im)
    return out.reshape(1, S, 2 * D)
```

```python
import jax
import jax.numpy as jnp
from jax import lax
import jax.experimental.pallas as pl
import jax.experimental.pallas.tpu as pltpu

S = 2048
D = 448
DP = 512
HD = D // 2
H = 16
DH = 28
W = 8
DIL = 2
NJ = 16
NL = 128
OG = 2
XS = NJ + 1
OS = 24
PLAN = ((13, "a", 0, 112), (27, "a", 112, 224), (28, "a", 224, 448), (28, "y", 0, 448))
F32 = jnp.float32
BF16 = jnp.bfloat16
U32 = jnp.uint32


def _cmul(ar, ai, br, bi):
    return ar * br - ai * bi, ar * bi + ai * br


def _col_bcast(row):
    return jnp.broadcast_to(row, (128, DP)).T[:D]


def _min(a, b):
    return min(a, b) if isinstance(a, int) else jnp.minimum(a, b)


def _mult(a, n):
    return a if isinstance(a, int) else pl.multiple_of(a, n)


def _pack(v):
    return pltpu.bitcast(v.astype(BF16), U32)


def _bf(v):
    return pltpu.bitcast(v, BF16)


def _stage_x(raw_ref, xt_ref, c):
    cols = pl.ds(_mult(128 * c, 128), 128)
    head = pltpu.bitcast(raw_ref[0:256, cols], U32).T
    tail = jnp.concatenate(
        [pltpu.bitcast(raw_ref[256:D, cols], U32), jnp.zeros(((DP - D) // 2, 128), U32)], axis=0)
    tail = tail.T
    for i in range(128 // NJ):
        dst = pl.ds(c * (128 // NJ * XS) + i * XS, NJ)
        xt_ref[0, dst, :] = head[NJ * i:NJ * i + NJ]
        xt_ref[1, dst, :] = tail[NJ * i:NJ * i + NJ]


def _gather_x(xt_ref, xp_ref, j):
    for h in range(2):
        xp_ref[j, 128 * h:128 * h + 128] = xt_ref[h, pl.ds(j, NL, stride=XS), :].T


def _kernel(lre_ref, lim_ref, ldt_ref, dsk_ref,
            ax_hbm, wqkv_hbm, wo_hbm, bx_hbm, bre_hbm, bim_hbm, cre_hbm, cim_hbm,
            out_hbm,
            xa_raw, xb_raw, wqkv_raw, wo_raw, bre_raw, bim_raw, cre_raw, cim_raw,
            xa_t, xb_t, xa_p, xb_p, bbar, cc, wt32, wt, wo32, wot,
            lam_r, lam_i, dsk, bu, st, et, ct, ht, qt, kk, vv, ot, res, stage,
            in_sems, out_sems):
    cp_bre = pltpu.make_async_copy(bre_hbm, bre_raw, in_sems.at[0])
    cp_bim = pltpu.make_async_copy(bim_hbm, bim_raw, in_sems.at[1])
    cp_bx = [pltpu.make_async_copy(bx_hbm.at[:, pl.ds(512 * i, 512)],
                                   xb_raw.at[:, pl.ds(512 * i, 512)], in_sems.at[8 + i])
             for i in range(4)]
    cp_wqkv = pltpu.make_async_copy(wqkv_hbm, wqkv_raw, in_sems.at[3])
    cp_ax = pltpu.make_async_copy(ax_hbm, xa_raw, in_sems.at[4])
    cp_cre = pltpu.make_async_copy(cre_hbm, cre_raw, in_sems.at[5])
    cp_cim = pltpu.make_async_copy(cim_hbm, cim_raw, in_sems.at[6])
    cp_wo = pltpu.make_async_copy(wo_hbm, wo_raw, in_sems.at[7])
    for c in (*cp_bx[:2], cp_bre, cp_bim, *cp_bx[2:], cp_wqkv, cp_ax, cp_cre, cp_cim, cp_wo):
        c.start()

    def row(ref):
        v = ref[...].astype(F32).reshape(1, D)
        return jnp.concatenate([v, jnp.ones((1, DP - D), F32)], axis=1)

    lr, li = row(lre_ref), row(lim_ref)
    dt = jnp.exp(row(ldt_ref)).astype(BF16).astype(F32)
    mag = jnp.exp(dt * lr)
    ar, ai = mag * jnp.cos(dt * li), mag * jnp.sin(dt * li)
    den = lr * lr + li * li
    cr = ((ar - 1.0) * lr + ai * li) / den
    ci = (ai * lr - (ar - 1.0) * li) / den
    lam_r[...] = _col_bcast(ar)
    lam_i[...] = _col_bcast(ai)
    valid = lax.broadcasted_iota(jnp.int32, (1, DP), 1) < D
    pr, pi = jnp.where(valid, ar, 0.0), jnp.where(valid, ai, 0.0)
    for _ in range(4):
        pr, pi = _cmul(pr, pi, pr, pi)
    blocks = lambda v: [v[:, 128 * i:128 * i + 128] for i in range(4)]
    pw_a = jnp.concatenate(blocks(pr) + blocks(pr), axis=0)
    pw_b = jnp.concatenate(blocks(-pi) + blocks(pi), axis=0)

    zcol = jnp.zeros((D, DP - D), F32)

    def make_bbar(g):
        for part, raw in enumerate((bre_raw, bim_raw)):
            u = pltpu.bitcast(raw[64 * g:64 * g + 64], U32)
            bbar[64 * g + 32 * part:64 * g + 32 * part + 32] = jnp.concatenate(
                [u, jnp.zeros((32, DP - D), U32)], axis=1)

    for i in range(4):
        cp_bx[i].wait()
        if i == 2:
            cp_bre.wait()
            cp_bim.wait()
        for c in range(4 * i, 4 * i + 4):
            _stage_x(xb_raw, xb_t, c)
        if i == 2:
            for g in range(7):
                make_bbar(g)
    _gather_x(xb_t, xb_p, 0)

    def scan_group(g, src, j_out):
        ro, io = 128 * g, 128 * g + 64
        a_r, a_i = lam_r[64 * g:64 * g + 64], lam_i[64 * g:64 * g + 64]
        p_r, p_i = _cmul(a_r, a_i, st[ro:ro + 64], st[io:io + 64])
        n_r = p_r + src(ro)
        n_i = p_i + src(io)
        st[ro:ro + 64] = n_r
        st[io:io + 64] = n_i
        if j_out is not None:
            ht[j_out, ro // 2:ro // 2 + 32] = _pack(n_r)
            ht[j_out, io // 2:io // 2 + 32] = _pack(n_i)

    st[...] = jnp.zeros((2 * D, NL), F32)

    def p1_base(j):
        x = _bf(xb_p[j])
        _gather_x(xb_t, xb_p, _min(j + 1, NJ - 1))
        res = jnp.dot(_bf(bbar[...]), x, preferred_element_type=F32)
        bu[j] = res
        for g in range(7):
            scan_group(g, lambda o: res[o:o + 64], None)

    def wqkv_transpose(lo):
        blk = jnp.concatenate(
            [wqkv_raw[:, pl.ds(lo, 128)].astype(F32), jnp.zeros((DP - D, 128), F32)], axis=0)
        for kb in range(4):
            wt32[kb, pl.ds(lo, 128), :] = blk[128 * kb:128 * kb + 128].T

    def wqkv_gather(idx):
        src = (idx // DH) * D + idx % DH
        dst = pl.ds(_mult(idx * (H // 2), H // 2), H // 2)
        for kb in range(4):
            wt[dst, 128 * kb:128 * kb + 128] = _pack(wt32[kb, pl.ds(src, H, stride=DH), :])

    for j in range(6):
        p1_base(j)
    cp_wqkv.wait()

    for i in range(5):
        p1_base(i + 6)
        for u in range(2):
            wqkv_transpose(_mult(256 * i + 128 * u, 128))

    tail = jnp.concatenate(
        [wqkv_raw[:, 1280:3 * D].astype(F32), jnp.zeros((D, 64), F32)], axis=1)
    tail = jnp.concatenate([tail, jnp.zeros((DP - D, 128), F32)], axis=0)
    for kb in range(4):
        wt32[kb, 1280:1408, :] = tail[128 * kb:128 * kb + 128].T
    cp_ax.wait()

    for i in range(5):
        p1_base(i + 11)
        for u in range(17):
            wqkv_gather(_min(17 * i + u, 3 * DH - 1))
        for u in range(3):
            _stage_x(xa_raw, xa_t, 3 * i + u)

    cp_cre.wait()
    cp_cim.wait()
    _stage_x(xa_raw, xa_t, 15)
    _gather_x(xa_t, xa_p, 0)

    lane_d = lax.broadcasted_iota(jnp.int32, (HD, NL), 1)

    def qkv(j, filler):
        x = _bf(xa_p[j])
        if j + 1 < NJ:
            _gather_x(xa_t, xa_p, j + 1)
        js = (j + 30) % 32
        for i, (t, h) in enumerate(((1, 0), (1, 1), (2, 0), (2, 1), (0, 0), (0, 1))):
            r0 = (t * D + h * HD) // 2
            res = jnp.dot(_bf(wt[r0:r0 + HD // 2]), x, preferred_element_type=F32)
            rows = slice(h * HD, (h + 1) * HD)
            if t == 0:
                qt[j, rows] = res
            elif t == 1:
                kk[j + 14, rows] = res
                kk[js, rows] = pltpu.roll(res, 1, 1)
            else:
                vv[j + 14, rows] = res
                vv[js, rows] = jnp.where(lane_d == 0, vv[14, rows], pltpu.roll(res, 1, 1))
            filler(i)

    qkv(0, lambda i: None)
    z64 = jnp.zeros((64, NL), F32)
    for b in range(4):
        for part in range(2):
            lo = st[256 * b + 64 * part:256 * b + 64 * part + 64]
            hi = st[256 * b + 128 + 64 * part:256 * b + 192 + 64 * part] if b < 3 else z64
            et[512 * part + 128 * b:512 * part + 128 * b + 128] = jnp.concatenate([lo, hi], axis=0).T
    c = jnp.zeros((8, 128), F32)
    for l in range(NL):
        ct[pl.ds(l, 8, stride=NL), :] = c
        if l < NL - 1:
            c = (pw_a * c + et[pl.ds(l, 8, stride=NL), :]) + pw_b * pltpu.roll(c, 4, 0)
    for b in range(4):
        for part in range(2):
            t = ct[512 * part + 128 * b:512 * part + 128 * b + 128].T
            st[256 * b + 64 * part:256 * b + 64 * part + 64] = t[0:64]
            if b < 3:
                st[256 * b + 128 + 64 * part:256 * b + 192 + 64 * part] = t[64:128]

    dsk[...] = _col_bcast(row(dsk_ref))

    def make_cc(r):
        x_r, x_i = cre_raw[r:r + 64].astype(F32), cim_raw[r:r + 64].astype(F32)
        g_r, g_i = 2.0 * cr[:, :D], 2.0 * ci[:, :D]
        c_r = _pack(g_r * x_r - g_i * x_i)
        c_i = _pack(-(g_r * x_i + g_i * x_r))
        for g in range(7):
            cc[r // 2:r // 2 + 32, 128 * g:128 * g + 128] = jnp.concatenate(
                [c_r[:, 64 * g:64 * g + 64], c_i[:, 64 * g:64 * g + 64]], axis=1)

    for j in range(1, NJ):
        def filler(i):
            for g in ((0, 1), (2,), (3,), (4,), (5,), (6,))[i]:
                scan_group(g, lambda o: bu[j - 1, o:o + 64], j - 1)
        qkv(j, filler)
        if j % 2 == 0:
            make_cc(32 * (j - 2))

    for g in range(7):
        scan_group(g, lambda o: bu[NJ - 1, o:o + 64], NJ - 1)
    cp_wo.wait()
    wo_p = jnp.concatenate([wo_raw[...].astype(F32), zcol], axis=1)
    for kb in range(4):
        wt32[kb, 0:D, :] = wo_p[:, 128 * kb:128 * kb + 128]
        for d in range(DH):
            wo32[d * H:(d + 1) * H, 128 * kb:128 * kb + 128] = wt32[kb, pl.ds(d, H, stride=DH), :]
    wo32[D:DP, :] = jnp.zeros((DP - D, DP), F32)
    wot[...] = _pack(wo32[...].T[:D])
    ot[D // 2:DP // 2] = jnp.zeros(((DP - D) // 2, NL), U32)

    lane_h = lax.broadcasted_iota(jnp.int32, (H, NL), 1)
    scale = DH ** -0.5

    def out_copies(i):
        rows = pl.ds(i * OG, OG)
        return [pltpu.make_async_copy(stage.at[c, :, rows, :],
                                      out_hbm.at[:, rows, pl.ds(128 * c, 128)],
                                      out_sems.at[i * 7 + c]) for c in range(7)]

    def attend(j, fill_qk, fill_pv):
        acc = [None] * W
        for d in range(DH):
            q = qt[j, d * H:(d + 1) * H]
            for w in range(W):
                t = q * kk[j + 14 - DIL * w, d * H:(d + 1) * H]
                acc[w] = t if d == 0 else acc[w] + t
            fill_qk(d)
        lg = [jnp.where((lane_h == 0) & (j < DIL * w), -1e9, acc[w] * scale) for w in range(W)]
        m = lg[0]
        for w in range(1, W):
            m = jnp.maximum(m, lg[w])
        e = [jnp.exp(l - m) for l in lg]
        tot = e[0]
        for w in range(1, W):
            tot = tot + e[w]
        inv = 1.0 / tot
        p = [x * inv for x in e]
        for d in range(DH):
            fill_pv(d)
            o = p[0] * vv[j + 14, d * H:(d + 1) * H]
            for w in range(1, W):
                o = o + p[w] * vv[j + 14 - DIL * w, d * H:(d + 1) * H]
            ot[d * (H // 2):(d + 1) * (H // 2)] = _pack(o)

    def ssm_out(j, lo, hi):
        rows = slice(lo, hi)
        prow = slice(lo // 2, hi // 2)
        y = jnp.dot(_bf(cc[prow]), _bf(ht[j]), preferred_element_type=F32)
        res[j % 2, rows] = y + _bf(xb_p[j, prow]).astype(F32) * dsk[rows]

    def att_out(j, lo, hi):
        prow = slice(lo // 2, hi // 2)
        qt[NJ + j % 2, lo:hi] = jnp.dot(_bf(wot[prow]), _bf(ot[...]), preferred_element_type=F32)

    def emit(j, c):
        a = j % 2
        if c < 3:
            blk = qt[NJ + a, 128 * c:128 * c + 128]
        elif c == 3:
            blk = jnp.concatenate([qt[NJ + a, 384:D], res[a, 0:64]], axis=0)
        else:
            blk = res[a, 128 * c - D:128 * c + 128 - D]
        stage.at[c].reshape(NL * OS, 128)[pl.ds(j, NL, stride=OS), :] = blk.T

    def send(j):
        @pl.when((j % OG == OG - 1) & (j >= 0))
        def _():
            for cp in out_copies(j // OG):
                cp.start()

    res[1] = jnp.zeros((D, NL), F32)
    qt[NJ + 1] = jnp.zeros((D, NL), F32)
    attend(0, lambda d: None, lambda d: ssm_out(0, 16 * d, 16 * d + HD) if d % 14 == 0 else None)

    @pl.loop(1, NJ)
    def _(j):
        def fill_qk(d):
            if d == 0:
                for c in range(7):
                    emit((j + NJ - 2) % NJ, c)
            fill_pv(d - DH)

        def fill_pv(d):
            for pos, kind, lo, hi in PLAN:
                if pos == d + DH:
                    if kind == "a":
                        att_out(j - 1, lo, hi)
                    else:
                        ssm_out(j, lo, hi)

        attend(j, fill_qk, fill_pv)
        send(j - 2)

    last = out_copies(NJ // OG - 1)
    for c in (4, 5, 6):
        emit(NJ - 2, c)
        emit(NJ - 1, c)
        last[c].start()
    att_out(NJ - 1, 0, D)
    for c in range(4):
        emit(NJ - 2, c)
    for c in range(4):
        emit(NJ - 1, c)
        last[c].start()
    for i in range(NJ // OG):
        for cp in out_copies(i):
            cp.wait()


@jax.jit
def pallas_concat_heads__sliding_local_dilated__ssm_conv_s5__prompt_kernel(
    A_x, A_wqkv, A_wo, B_x, B_Lambda_re, B_Lambda_im, B_B_re, B_B_im, B_C_re, B_C_im,
    B_log_dt, B_Dskip,
):
    vm = pl.BlockSpec(memory_space=pltpu.VMEM)
    hbm = pl.BlockSpec(memory_space=pltpu.HBM)
    out = pl.pallas_call(
        _kernel,
        in_specs=[vm] * 4 + [hbm] * 8,
        out_specs=hbm,
        out_shape=jax.ShapeDtypeStruct((NL, NJ, 2 * D), F32),
        scratch_shapes=[
            pltpu.VMEM((D, S), BF16), pltpu.VMEM((D, S), BF16),
            pltpu.VMEM((D, 3 * D), BF16), pltpu.VMEM((D, D), BF16),
            pltpu.VMEM((D, D), BF16), pltpu.VMEM((D, D), BF16),
            pltpu.VMEM((D, D), BF16), pltpu.VMEM((D, D), BF16),
            pltpu.VMEM((2, NL * XS, 128), U32), pltpu.VMEM((2, NL * XS, 128), U32),
            pltpu.VMEM((NJ, DP // 2, NL), U32), pltpu.VMEM((NJ, DP // 2, NL), U32),
            pltpu.VMEM((D, DP), U32), pltpu.VMEM((D // 2, 2 * D), U32),
            pltpu.VMEM((4, 1408, 128), F32), pltpu.VMEM((3 * D // 2, DP), U32),
            pltpu.VMEM((DP, DP), F32), pltpu.VMEM((D // 2, DP), U32),
            pltpu.VMEM((D, NL), F32), pltpu.VMEM((D, NL), F32), pltpu.VMEM((D, NL), F32),
            pltpu.VMEM((NJ, 2 * D, NL), F32), pltpu.VMEM((2 * D, NL), F32),
            pltpu.VMEM((8 * NL, 128), F32), pltpu.VMEM((8 * NL, 128), F32),
            pltpu.VMEM((NJ, D, NL), U32),
            pltpu.VMEM((NJ + 2, D, NL), F32), pltpu.VMEM((32, D, NL), F32),
            pltpu.VMEM((32, D, NL), F32), pltpu.VMEM((DP // 2, NL), U32),
            pltpu.VMEM((2, D, NL), F32),
            pltpu.VMEM((7, NL, OS, 128), F32),
            pltpu.SemaphoreType.DMA((16,)), pltpu.SemaphoreType.DMA((7 * NJ // OG,)),
        ],
        compiler_params=pltpu.CompilerParams(vmem_limit_bytes=100 * 1024 * 1024),
    )(B_Lambda_re, B_Lambda_im, B_log_dt, B_Dskip,
      A_x[0].T, A_wqkv, A_wo, B_x[0].T, B_B_re, B_B_im, B_C_re, B_C_im)
    return out.reshape(1, S, 2 * D)
```

```python
import jax
import jax.numpy as jnp
from jax import lax
import jax.experimental.pallas as pl
import jax.experimental.pallas.tpu as pltpu

S = 2048
D = 448
DP = 512
HD = D // 2
H = 16
DH = 28
W = 8
DIL = 2
NJ = 16
NL = 128
OG = 2
XS = NJ + 1
OS = 24
PLAN = ((13, "a", 0, 112), (27, "a", 112, 224), (28, "a", 224, 448), (28, "y", 0, 448))
LATE = 2
F32 = jnp.float32
BF16 = jnp.bfloat16
U32 = jnp.uint32


def _cmul(ar, ai, br, bi):
    return ar * br - ai * bi, ar * bi + ai * br


def _col_bcast(row):
    return jnp.broadcast_to(row, (128, DP)).T[:D]


def _min(a, b):
    return min(a, b) if isinstance(a, int) else jnp.minimum(a, b)


def _mult(a, n):
    return a if isinstance(a, int) else pl.multiple_of(a, n)


def _pack(v):
    return pltpu.bitcast(v.astype(BF16), U32)


def _bf(v):
    return pltpu.bitcast(v, BF16)


def _stage_x(raw_ref, xt_ref, c):
    cols = pl.ds(_mult(128 * c, 128), 128)
    head = pltpu.bitcast(raw_ref[0:256, cols], U32).T
    tail = jnp.concatenate(
        [pltpu.bitcast(raw_ref[256:D, cols], U32), jnp.zeros(((DP - D) // 2, 128), U32)], axis=0)
    tail = tail.T
    for i in range(128 // NJ):
        dst = pl.ds(c * (128 // NJ * XS) + i * XS, NJ)
        xt_ref[0, dst, :] = head[NJ * i:NJ * i + NJ]
        xt_ref[1, dst, :] = tail[NJ * i:NJ * i + NJ]


def _gather_x(xt_ref, xp_ref, j):
    for h in range(2):
        xp_ref[j, 128 * h:128 * h + 128] = xt_ref[h, pl.ds(j, NL, stride=XS), :].T


def _kernel(lre_ref, lim_ref, ldt_ref, dsk_ref,
            ax_hbm, wqkv_hbm, wo_hbm, bx_hbm, bre_hbm, bim_hbm, cre_hbm, cim_hbm,
            out_hbm,
            xa_raw, xb_raw, wqkv_raw, wo_raw, bre_raw, bim_raw, cre_raw, cim_raw,
            xa_t, xb_t, xa_p, xb_p, bbar, cc, wt32, wt, wo32, wot,
            lam_r, lam_i, dsk, bu, st, et, ct, ht, qt, kk, vv, ot, res, stage,
            in_sems, out_sems):
    cp_bre = pltpu.make_async_copy(bre_hbm, bre_raw, in_sems.at[0])
    cp_bim = pltpu.make_async_copy(bim_hbm, bim_raw, in_sems.at[1])
    cp_bx = [pltpu.make_async_copy(bx_hbm.at[:, pl.ds(512 * i, 512)],
                                   xb_raw.at[:, pl.ds(512 * i, 512)], in_sems.at[8 + i])
             for i in range(4)]
    cp_wqkv = pltpu.make_async_copy(wqkv_hbm, wqkv_raw, in_sems.at[3])
    cp_ax = pltpu.make_async_copy(ax_hbm, xa_raw, in_sems.at[4])
    cp_cre = pltpu.make_async_copy(cre_hbm, cre_raw, in_sems.at[5])
    cp_cim = pltpu.make_async_copy(cim_hbm, cim_raw, in_sems.at[6])
    cp_wo = pltpu.make_async_copy(wo_hbm, wo_raw, in_sems.at[7])
    for c in (*cp_bx[:2], cp_bre, cp_bim, *cp_bx[2:]):
        c.start()

    def row(ref):
        v = ref[...].astype(F32).reshape(1, D)
        return jnp.concatenate([v, jnp.ones((1, DP - D), F32)], axis=1)

    lr, li = row(lre_ref), row(lim_ref)
    dt = jnp.exp(row(ldt_ref)).astype(BF16).astype(F32)
    mag = jnp.exp(dt * lr)
    ar, ai = mag * jnp.cos(dt * li), mag * jnp.sin(dt * li)
    den = lr * lr + li * li
    cr = ((ar - 1.0) * lr + ai * li) / den
    ci = (ai * lr - (ar - 1.0) * li) / den
    lam_r[...] = _col_bcast(ar)
    lam_i[...] = _col_bcast(ai)
    valid = lax.broadcasted_iota(jnp.int32, (1, DP), 1) < D
    pr, pi = jnp.where(valid, ar, 0.0), jnp.where(valid, ai, 0.0)
    for _ in range(4):
        pr, pi = _cmul(pr, pi, pr, pi)
    blocks = lambda v: [v[:, 128 * i:128 * i + 128] for i in range(4)]
    pw_a = jnp.concatenate(blocks(pr) + blocks(pr), axis=0)
    pw_b = jnp.concatenate(blocks(-pi) + blocks(pi), axis=0)

    zcol = jnp.zeros((D, DP - D), F32)

    def make_bbar(g):
        for part, raw in enumerate((bre_raw, bim_raw)):
            u = pltpu.bitcast(raw[64 * g:64 * g + 64], U32)
            bbar[64 * g + 32 * part:64 * g + 32 * part + 32] = jnp.concatenate(
                [u, jnp.zeros((32, DP - D), U32)], axis=1)

    for i in range(4):
        cp_bx[i].wait()
        if i == LATE:
            for cp in (cp_wqkv, cp_ax, cp_cre, cp_cim, cp_wo):
                cp.start()
        if i == 2:
            cp_bre.wait()
            cp_bim.wait()
        for c in range(4 * i, 4 * i + 4):
            _stage_x(xb_raw, xb_t, c)
        if i == 2:
            for g in range(7):
                make_bbar(g)
    _gather_x(xb_t, xb_p, 0)

    def scan_group(g, src, j_out):
        ro, io = 128 * g, 128 * g + 64
        a_r, a_i = lam_r[64 * g:64 * g + 64], lam_i[64 * g:64 * g + 64]
        p_r, p_i = _cmul(a_r, a_i, st[ro:ro + 64], st[io:io + 64])
        n_r = p_r + src(ro)
        n_i = p_i + src(io)
        st[ro:ro + 64] = n_r
        st[io:io + 64] = n_i
        if j_out is not None:
            ht[j_out, ro // 2:ro // 2 + 32] = _pack(n_r)
            ht[j_out, io // 2:io // 2 + 32] = _pack(n_i)

    st[...] = jnp.zeros((2 * D, NL), F32)

    def p1_base(j):
        x = _bf(xb_p[j])
        _gather_x(xb_t, xb_p, _min(j + 1, NJ - 1))
        res = jnp.dot(_bf(bbar[...]), x, preferred_element_type=F32)
        bu[j] = res
        for g in range(7):
            scan_group(g, lambda o: res[o:o + 64], None)

    def wqkv_transpose(lo):
        blk = jnp.concatenate(
            [wqkv_raw[:, pl.ds(lo, 128)].astype(F32), jnp.zeros((DP - D, 128), F32)], axis=0)
        for kb in range(4):
            wt32[kb, pl.ds(lo, 128), :] = blk[128 * kb:128 * kb + 128].T

    def wqkv_gather(idx):
        src = (idx // DH) * D + idx % DH
        dst = pl.ds(_mult(idx * (H // 2), H // 2), H // 2)
        for kb in range(4):
            wt[dst, 128 * kb:128 * kb + 128] = _pack(wt32[kb, pl.ds(src, H, stride=DH), :])

    for j in range(6):
        p1_base(j)
    cp_wqkv.wait()

    for i in range(5):
        p1_base(i + 6)
        for u in range(2):
            wqkv_transpose(_mult(256 * i + 128 * u, 128))

    tail = jnp.concatenate(
        [wqkv_raw[:, 1280:3 * D].astype(F32), jnp.zeros((D, 64), F32)], axis=1)
    tail = jnp.concatenate([tail, jnp.zeros((DP - D, 128), F32)], axis=0)
    for kb in range(4):
        wt32[kb, 1280:1408, :] = tail[128 * kb:128 * kb + 128].T
    cp_ax.wait()

    for i in range(5):
        p1_base(i + 11)
        for u in range(17):
            wqkv_gather(_min(17 * i + u, 3 * DH - 1))
        for u in range(3):
            _stage_x(xa_raw, xa_t, 3 * i + u)

    cp_cre.wait()
    cp_cim.wait()
    _stage_x(xa_raw, xa_t, 15)
    _gather_x(xa_t, xa_p, 0)

    lane_d = lax.broadcasted_iota(jnp.int32, (HD, NL), 1)

    def qkv(j, filler):
        x = _bf(xa_p[j])
        if j + 1 < NJ:
            _gather_x(xa_t, xa_p, j + 1)
        js = (j + 30) % 32
        for i, (t, h) in enumerate(((1, 0), (1, 1), (2, 0), (2, 1), (0, 0), (0, 1))):
            r0 = (t * D + h * HD) // 2
            res = jnp.dot(_bf(wt[r0:r0 + HD // 2]), x, preferred_element_type=F32)
            rows = slice(h * HD, (h + 1) * HD)
            if t == 0:
                qt[j, rows] = res
            elif t == 1:
                kk[j + 14, rows] = res
                kk[js, rows] = pltpu.roll(res, 1, 1)
            else:
                vv[j + 14, rows] = res
                vv[js, rows] = jnp.where(lane_d == 0, vv[14, rows], pltpu.roll(res, 1, 1))
            filler(i)

    qkv(0, lambda i: None)
    z64 = jnp.zeros((64, NL), F32)
    for b in range(4):
        for part in range(2):
            lo = st[256 * b + 64 * part:256 * b + 64 * part + 64]
            hi = st[256 * b + 128 + 64 * part:256 * b + 192 + 64 * part] if b < 3 else z64
            et[512 * part + 128 * b:512 * part + 128 * b + 128] = jnp.concatenate([lo, hi], axis=0).T
    c = jnp.zeros((8, 128), F32)
    for l in range(NL):
        ct[pl.ds(l, 8, stride=NL), :] = c
        if l < NL - 1:
            c = (pw_a * c + et[pl.ds(l, 8, stride=NL), :]) + pw_b * pltpu.roll(c, 4, 0)
    for b in range(4):
        for part in range(2):
            t = ct[512 * part + 128 * b:512 * part + 128 * b + 128].T
            st[256 * b + 64 * part:256 * b + 64 * part + 64] = t[0:64]
            if b < 3:
                st[256 * b + 128 + 64 * part:256 * b + 192 + 64 * part] = t[64:128]

    dsk[...] = _col_bcast(row(dsk_ref))

    def make_cc(r):
        x_r, x_i = cre_raw[r:r + 64].astype(F32), cim_raw[r:r + 64].astype(F32)
        g_r, g_i = 2.0 * cr[:, :D], 2.0 * ci[:, :D]
        c_r = _pack(g_r * x_r - g_i * x_i)
        c_i = _pack(-(g_r * x_i + g_i * x_r))
        for g in range(7):
            cc[r // 2:r // 2 + 32, 128 * g:128 * g + 128] = jnp.concatenate(
                [c_r[:, 64 * g:64 * g + 64], c_i[:, 64 * g:64 * g + 64]], axis=1)

    for j in range(1, NJ):
        def filler(i):
            for g in ((0, 1), (2,), (3,), (4,), (5,), (6,))[i]:
                scan_group(g, lambda o: bu[j - 1, o:o + 64], j - 1)
        qkv(j, filler)
        if j % 2 == 0:
            make_cc(32 * (j - 2))

    for g in range(7):
        scan_group(g, lambda o: bu[NJ - 1, o:o + 64], NJ - 1)
    cp_wo.wait()
    wo_p = jnp.concatenate([wo_raw[...].astype(F32), zcol], axis=1)
    for kb in range(4):
        wt32[kb, 0:D, :] = wo_p[:, 128 * kb:128 * kb + 128]
        for d in range(DH):
            wo32[d * H:(d + 1) * H, 128 * kb:128 * kb + 128] = wt32[kb, pl.ds(d, H, stride=DH), :]
    wo32[D:DP, :] = jnp.zeros((DP - D, DP), F32)
    wot[...] = _pack(wo32[...].T[:D])
    ot[D // 2:DP // 2] = jnp.zeros(((DP - D) // 2, NL), U32)

    lane_h = lax.broadcasted_iota(jnp.int32, (H, NL), 1)
    scale = DH ** -0.5

    def out_copies(i):
        rows = pl.ds(i * OG, OG)
        return [pltpu.make_async_copy(stage.at[c, :, rows, :],
                                      out_hbm.at[:, rows, pl.ds(128 * c, 128)],
                                      out_sems.at[i * 7 + c]) for c in range(7)]

    def attend(j, fill_qk, fill_pv):
        acc = [None] * W
        for d in range(DH):
            q = qt[j, d * H:(d + 1) * H]
            for w in range(W):
                t = q * kk[j + 14 - DIL * w, d * H:(d + 1) * H]
                acc[w] = t if d == 0 else acc[w] + t
            fill_qk(d)
        lg = [jnp.where((lane_h == 0) & (j < DIL * w), -1e9, acc[w] * scale) for w in range(W)]
        m = lg[0]
        for w in range(1, W):
            m = jnp.maximum(m, lg[w])
        e = [jnp.exp(l - m) for l in lg]
        tot = e[0]
        for w in range(1, W):
            tot = tot + e[w]
        inv = 1.0 / tot
        p = [x * inv for x in e]
        for d in range(DH):
            fill_pv(d)
            o = p[0] * vv[j + 14, d * H:(d + 1) * H]
            for w in range(1, W):
                o = o + p[w] * vv[j + 14 - DIL * w, d * H:(d + 1) * H]
            ot[d * (H // 2):(d + 1) * (H // 2)] = _pack(o)

    def ssm_out(j, lo, hi):
        rows = slice(lo, hi)
        prow = slice(lo // 2, hi // 2)
        y = jnp.dot(_bf(cc[prow]), _bf(ht[j]), preferred_element_type=F32)
        res[j % 2, rows] = y + _bf(xb_p[j, prow]).astype(F32) * dsk[rows]

    def att_out(j, lo, hi):
        prow = slice(lo // 2, hi // 2)
        qt[NJ + j % 2, lo:hi] = jnp.dot(_bf(wot[prow]), _bf(ot[...]), preferred_element_type=F32)

    def emit(j, c):
        a = j % 2
        if c < 3:
            blk = qt[NJ + a, 128 * c:128 * c + 128]
        elif c == 3:
            blk = jnp.concatenate([qt[NJ + a, 384:D], res[a, 0:64]], axis=0)
        else:
            blk = res[a, 128 * c - D:128 * c + 128 - D]
        stage.at[c].reshape(NL * OS, 128)[pl.ds(j, NL, stride=OS), :] = blk.T

    def send(j):
        @pl.when((j % OG == OG - 1) & (j >= 0))
        def _():
            for cp in out_copies(j // OG):
                cp.start()

    res[1] = jnp.zeros((D, NL), F32)
    qt[NJ + 1] = jnp.zeros((D, NL), F32)
    attend(0, lambda d: None, lambda d: ssm_out(0, 16 * d, 16 * d + HD) if d % 14 == 0 else None)

    @pl.loop(1, NJ)
    def _(j):
        def fill_qk(d):
            if d == 0:
                for c in range(7):
                    emit((j + NJ - 2) % NJ, c)
            fill_pv(d - DH)

        def fill_pv(d):
            for pos, kind, lo, hi in PLAN:
                if pos == d + DH:
                    if kind == "a":
                        att_out(j - 1, lo, hi)
                    else:
                        ssm_out(j, lo, hi)

        attend(j, fill_qk, fill_pv)
        send(j - 2)

    last = out_copies(NJ // OG - 1)
    for c in (4, 5, 6):
        emit(NJ - 2, c)
        emit(NJ - 1, c)
        last[c].start()
    att_out(NJ - 1, 0, D)
    for c in range(4):
        emit(NJ - 2, c)
    for c in range(4):
        emit(NJ - 1, c)
        last[c].start()
    for i in range(NJ // OG):
        for cp in out_copies(i):
            cp.wait()


@jax.jit
def pallas_concat_heads__sliding_local_dilated__ssm_conv_s5__prompt_kernel(
    A_x, A_wqkv, A_wo, B_x, B_Lambda_re, B_Lambda_im, B_B_re, B_B_im, B_C_re, B_C_im,
    B_log_dt, B_Dskip,
):
    vm = pl.BlockSpec(memory_space=pltpu.VMEM)
    hbm = pl.BlockSpec(memory_space=pltpu.HBM)
    out = pl.pallas_call(
        _kernel,
        in_specs=[vm] * 4 + [hbm] * 8,
        out_specs=hbm,
        out_shape=jax.ShapeDtypeStruct((NL, NJ, 2 * D), F32),
        scratch_shapes=[
            pltpu.VMEM((D, S), BF16), pltpu.VMEM((D, S), BF16),
            pltpu.VMEM((D, 3 * D), BF16), pltpu.VMEM((D, D), BF16),
            pltpu.VMEM((D, D), BF16), pltpu.VMEM((D, D), BF16),
            pltpu.VMEM((D, D), BF16), pltpu.VMEM((D, D), BF16),
            pltpu.VMEM((2, NL * XS, 128), U32), pltpu.VMEM((2, NL * XS, 128), U32),
            pltpu.VMEM((NJ, DP // 2, NL), U32), pltpu.VMEM((NJ, DP // 2, NL), U32),
            pltpu.VMEM((D, DP), U32), pltpu.VMEM((D // 2, 2 * D), U32),
            pltpu.VMEM((4, 1408, 128), F32), pltpu.VMEM((3 * D // 2, DP), U32),
            pltpu.VMEM((DP, DP), F32), pltpu.VMEM((D // 2, DP), U32),
            pltpu.VMEM((D, NL), F32), pltpu.VMEM((D, NL), F32), pltpu.VMEM((D, NL), F32),
            pltpu.VMEM((NJ, 2 * D, NL), F32), pltpu.VMEM((2 * D, NL), F32),
            pltpu.VMEM((8 * NL, 128), F32), pltpu.VMEM((8 * NL, 128), F32),
            pltpu.VMEM((NJ, D, NL), U32),
            pltpu.VMEM((NJ + 2, D, NL), F32), pltpu.VMEM((32, D, NL), F32),
            pltpu.VMEM((32, D, NL), F32), pltpu.VMEM((DP // 2, NL), U32),
            pltpu.VMEM((2, D, NL), F32),
            pltpu.VMEM((7, NL, OS, 128), F32),
            pltpu.SemaphoreType.DMA((16,)), pltpu.SemaphoreType.DMA((7 * NJ // OG,)),
        ],
        compiler_params=pltpu.CompilerParams(vmem_limit_bytes=100 * 1024 * 1024),
    )(B_Lambda_re, B_Lambda_im, B_log_dt, B_Dskip,
      A_x[0].T, A_wqkv, A_wo, B_x[0].T, B_B_re, B_B_im, B_C_re, B_C_im)
    return out.reshape(1, S, 2 * D)
```
